```python
import jax
import jax.numpy as jnp

def _softmax(x, axis=-1):
    return jax.nn.softmax(x, axis=axis)
def _gelu(x):
    return jax.nn.gelu(x, approximate=True)
def _silu(x):
    return jax.nn.silu(x)
def _sigmoid(x):
    return jax.nn.sigmoid(x)
def _layernorm(x, axis=-1, eps=1e-5):
    m = jnp.mean(x, axis=axis, keepdims=True)
    v = jnp.var(x, axis=axis, keepdims=True)
    return (x - m) / jnp.sqrt(v + eps)
def _scatter_add(tgt, idx, src, axis=0):
    return tgt.at[idx].add(src)
def _segment_sum(src, seg, n):
    return jax.ops.segment_sum(src, seg, n)
class _Rng:
    def __init__(self, key):
        self._k = key
    def _next(self):
        self._k, sub = jax.random.split(self._k)
        return sub
    def normal(self, shape):
        return jax.random.normal(self._next(), shape, dtype=jnp.bfloat16)
    def randint(self, lo, hi, shape):
        return jax.random.randint(self._next(), shape, lo, hi, dtype=jnp.int32)
    def uniform(self, shape, lo=0.0, hi=1.0):
        return jax.random.uniform(self._next(), shape, jnp.bfloat16, lo, hi)
    def permutation(self, n):
        return jax.random.permutation(self._next(), n)


kernel_name = 'interleave_layers__sliding_block_cached__moe_arch_mod__decode'

def setup_inputs():
    _rng = _Rng(jax.random.key(int.from_bytes(__import__("os").urandom(4), "little")))
    _w = (lambda a: (lambda t: t.astype(jnp.bfloat16) if jnp.issubdtype(t.dtype, jnp.floating) else t)(jnp.asarray(a)))
    def _A_setup():
        B, Sq, D = 4, 1, 640
        Hq, Hkv, Sk, Dh = 32, 32, 4096, 192
        assert Hq % Hkv == 0, (Hq, Hkv)
        return {
            "x": _w((lambda *s: _rng.normal(s) * 0.05)(B, Sq, D)),
            "k_cache": _w((lambda *s: _rng.normal(s) * 0.05)(B, Hkv, Sk, Dh)),
            "v_cache": _w((lambda *s: _rng.normal(s) * 0.05)(B, Hkv, Sk, Dh)),
            "wq": _w((lambda *s: _rng.normal(s) * 0.05)(D, Hq * Dh) * (D ** -0.5)),
            "wo": _w((lambda *s: _rng.normal(s) * 0.05)(Hq * Dh, D) * ((Hq * Dh) ** -0.5)),
        }
    _A_in = _A_setup()

    def _B_setup():
        B, S, D, F, C = 4, 1, 640, 1536, 1
        return {
            "x": _w((lambda *s: _rng.normal(s) * 0.05)(B, S, D)),
            "w_r": _w((lambda *s: _rng.normal(s) * 0.05)(D)),
            "w_gate": _w((lambda *s: _rng.normal(s) * 0.05)(D, F)),
            "w_up": _w((lambda *s: _rng.normal(s) * 0.05)(D, F)),
            "w_down": _w((lambda *s: _rng.normal(s) * 0.05)(F, D)),
        }
    _B_in = _B_setup()

    return {
        "A_x": _A_in["x"],
        "A_k_cache": _A_in["k_cache"],
        "A_v_cache": _A_in["v_cache"],
        "A_wq": _A_in["wq"],
        "A_wo": _A_in["wo"],
        "B_x": _B_in["x"],
        "B_w_r": _B_in["w_r"],
        "B_w_gate": _B_in["w_gate"],
        "B_w_up": _B_in["w_up"],
        "B_w_down": _B_in["w_down"],
    }

def reference(A_x, A_k_cache, A_v_cache, A_wq, A_wo, B_x, B_w_r, B_w_gate, B_w_up, B_w_down):
    def _A_ref(x, k_cache, v_cache, wq, wo):
        B, Sq, D = x.shape
        Hq, Dh = 32, 192
        Hkv, Sk = k_cache.shape[1], k_cache.shape[2]
        W = min(4096, max(256, Sk // 4))
        rep = Hq // Hkv
        q = (lambda x, *d: x.transpose(*d))((x @ wq).reshape(B, Sq, Hq, Dh), 0, 2, 1, 3)
        k = jnp.repeat(k_cache[:, :, Sk - W:, :], rep, axis=1)
        v = jnp.repeat(v_cache[:, :, Sk - W:, :], rep, axis=1)
        scores = jnp.einsum("bhqd,bhkd->bhqk", q, k) * (Dh ** -0.5)
        p = _softmax(scores, axis=-1)
        o = jnp.einsum("bhqk,bhkd->bhqd", p, v)
        return (lambda x, *d: x.transpose(*d))(o, 0, 2, 1, 3).reshape(B, Sq, Hq * Dh) @ wo

    def _B_ref(x, w_r, w_gate, w_up, w_down):
        B, S, D = x.shape
        C = 1
        r = x @ w_r
        idx = jnp.argsort(-r, axis=-1)[:, :C]
        idx_e = jnp.repeat(idx.reshape(B, C, 1), D, axis=2)
        x_sel = jnp.take_along_axis(x, idx_e, axis=1)
        g = _silu(x_sel @ w_gate)
        u = x_sel @ w_up
        y = (g * u) @ w_down
        r_sel = _sigmoid(jnp.take_along_axis(r, idx, axis=1))
        y = y * r_sel.reshape(B, C, 1)
        b_off = (jnp.arange(B) * S).reshape(B, 1)
        flat_idx = (idx + b_off).reshape(B * C)
        zero = (x * 0.0).reshape(B * S, D)
        upd = _scatter_add(zero, flat_idx, y.reshape(B * C, D), axis=0)
        return x + upd.reshape(B, S, D)

    x = A_x
    x = x + _A_ref(_layernorm(x, axis=-1), A_k_cache, A_v_cache, A_wq, A_wo)
    x = x + _B_ref(_layernorm(x, axis=-1), B_w_r, B_w_gate, B_w_up, B_w_down)
    x = x + _A_ref(_layernorm(x, axis=-1), A_k_cache, A_v_cache, A_wq, A_wo)
    x = x + _B_ref(_layernorm(x, axis=-1), B_w_r, B_w_gate, B_w_up, B_w_down)
    return x
```

```python
import functools

import jax
import jax.numpy as jnp
import numpy as np
from jax import lax
from jax.experimental import pallas as pl
from jax.experimental.pallas import tpu as pltpu

B, D, H, DH, S, F = 4, 640, 32, 192, 4096, 1536
W = min(4096, max(256, S // 4))
HD = H * DH
LANES = 128
NJ = W // LANES
NC = HD // LANES
ND = D // LANES
NF = F // LANES
EPS = 1e-5
SCALE = DH ** -0.5

G = 16
NG = H // G
CPG = G * DH // LANES
V_PIECES = (7, 4, 3, 2)
assert sum(V_PIECES) * 3 == NC

bf16 = jnp.bfloat16
f32 = jnp.float32


def _nn(a, b):
    return jnp.dot(a, b, preferred_element_type=f32)


def _nt(a, b):
    return lax.dot_general(a, b, (((1,), (1,)), ((), ())), preferred_element_type=f32)


def _layernorm(xs):
    tot = functools.reduce(jnp.add, xs)
    mean = jnp.sum(tot, axis=1, keepdims=True) * (1.0 / D)
    cs = [x - mean for x in xs]
    sq = functools.reduce(jnp.add, [c * c for c in cs])
    var = jnp.sum(sq, axis=1, keepdims=True) * (1.0 / D)
    inv = lax.rsqrt(var + EPS)
    return [c * inv for c in cs]


def _kernel(x_ref, wr_ref, kT, vT, wq_h, wo_h, wg_h, wu_h, wd_h, o_ref,
            kbuf, vbuf, wq, wo, wg, wu, wd, xs_ref, ys_ref, wsem, ksem, vsem):

    def k_copies(b):
        return [pltpu.make_async_copy(
            kT.at[b, :, pl.ds(S - W + LANES * j, LANES)], kbuf.at[b, j], ksem.at[b])
            for j in range(NJ)]

    def v_copies(b, p):
        t0 = 3 * sum(V_PIECES[:p])
        rows = pl.ds(t0 * LANES, 3 * V_PIECES[p] * LANES)
        return [pltpu.make_async_copy(
            vT.at[b, rows, pl.ds(S - W + LANES * j, LANES)], vbuf.at[b, j, rows], vsem.at[b, p])
            for j in range(NJ)]

    def strip_copies(src, dst, n, sem):
        return [pltpu.make_async_copy(src.at[:, pl.ds(LANES * c, LANES)], dst.at[c], sem)
                for c in range(n)]

    wq_c = strip_copies(wq_h, wq, NC, wsem.at[0])
    wo_c = strip_copies(wo_h, wo, ND, wsem.at[1])
    wg_c = strip_copies(wg_h, wg, NF, wsem.at[2])
    wu_c = strip_copies(wu_h, wu, NF, wsem.at[3])
    wd_c = strip_copies(wd_h, wd, ND, wsem.at[4])

    def start(cs):
        for c in cs:
            c.start()

    def wait(cs):
        for c in cs:
            c.wait()

    def start_kv(b):
        start(k_copies(b))
        for p in range(len(V_PIECES)):
            start(v_copies(b, p))

    start(wq_c)
    start(k_copies(0))

    xs_ref[...] = x_ref[...].astype(f32)
    wr = wr_ref[...].astype(f32)
    wr_t = [jnp.broadcast_to(wr[:, LANES * n:LANES * (n + 1)], (G, LANES)) for n in range(ND)]

    row = lax.broadcasted_iota(jnp.int32, (G, LANES), 0)
    lane = lax.broadcasted_iota(jnp.int32, (G, LANES), 1)

    def head_mask(c):
        col = lane + c * LANES
        lo = row * DH
        return (col >= lo) & (col < lo + DH)

    wait(wq_c)
    for p in range(len(V_PIECES)):
        start(v_copies(0, p))
    start(wo_c)
    start(wg_c)
    start(wu_c)
    start(wd_c)

    v_first_tile = {3 * sum(V_PIECES[:p]): p for p in range(len(V_PIECES))}

    def layer(b, xs, first):
        xn = [t.astype(bf16) for t in _layernorm(xs)]
        xnb = jnp.concatenate(xn, axis=1)
        if first:
            wait(k_copies(b))

            @pl.when(b + 1 < B)
            def _():
                start_kv(b + 1)

        acc_o = [None] * ND
        for g in range(NG):
            sc = [None] * NJ
            for c in range(CPG):
                cc = g * CPG + c
                qt = _nn(xnb, wq[cc])
                qt = jnp.where(head_mask(c), qt, 0.0).astype(bf16)
                for j in range(NJ):
                    t = _nn(qt, kbuf[b, j, pl.ds(cc * LANES, LANES), :])
                    sc[j] = t if sc[j] is None else sc[j] + t
            m = functools.reduce(jnp.maximum, sc)
            m = jnp.max(m, axis=1, keepdims=True)
            es = [jnp.exp((t - m) * SCALE) for t in sc]
            l = jnp.sum(functools.reduce(jnp.add, es), axis=1, keepdims=True)
            inv = 1.0 / l
            ps = [(e * inv).astype(bf16) for e in es]
            for c in range(CPG):
                cc = g * CPG + c
                if first and cc in v_first_tile:
                    wait(v_copies(b, v_first_tile[cc]))
                    if cc == 0:
                        @pl.when(b == 0)
                        def _():
                            wait(wo_c)
                ot = None
                for j in range(NJ):
                    t = _nt(ps[j], vbuf[b, j, pl.ds(cc * LANES, LANES), :])
                    ot = t if ot is None else ot + t
                ot = jnp.where(head_mask(c), ot, 0.0).astype(bf16)
                for n in range(ND):
                    t = _nn(ot, wo[n, pl.ds(cc * LANES, LANES), :])
                    acc_o[n] = t if acc_o[n] is None else acc_o[n] + t
        x1 = [x + jnp.sum(a, axis=0, keepdims=True) for x, a in zip(xs, acc_o)]

        if first:
            @pl.when(b == 0)
            def _():
                wait(wg_c)
                wait(wu_c)
                wait(wd_c)
        xn = _layernorm(x1)
        xnb_t = [t.astype(bf16) for t in xn]
        xnb = jnp.concatenate(xnb_t, axis=1)
        rr = functools.reduce(jnp.add, [a.astype(f32) * w for a, w in zip(xnb_t, wr_t)])
        r = jnp.sum(rr, axis=1, keepdims=True)
        gate = jax.nn.sigmoid(r)
        y = [None] * ND
        for f in range(NF):
            gt = _nn(xnb, wg[f])
            ut = _nn(xnb, wu[f])
            h = (gt * jax.nn.sigmoid(gt) * ut).astype(bf16)
            for n in range(ND):
                t = _nn(h, wd[n, pl.ds(f * LANES, LANES), :])
                y[n] = t if y[n] is None else y[n] + t
        return [a + bb + c * gate for a, bb, c in zip(x1, xn, y)]

    def batch(b, carry):
        x = jnp.broadcast_to(xs_ref[pl.ds(b, 1), :], (G, D))
        xs = [x[:, LANES * n:LANES * (n + 1)] for n in range(ND)]
        xs = layer(b, xs, True)
        xs = layer(b, xs, False)
        ys_ref[pl.ds(b, 1), :] = jnp.concatenate(xs, axis=1)[0:1, :]
        return carry

    lax.fori_loop(0, B, batch, 0)
    o_ref[...] = ys_ref[...].astype(o_ref.dtype)


@jax.jit
def pallas_interleave_layers__sliding_block_cached__moe_arch_mod__decode_kernel(
    A_x: jax.Array,
    A_k_cache: jax.Array,
    A_v_cache: jax.Array,
    A_wq: jax.Array,
    A_wo: jax.Array,
    B_x: jax.Array,
    B_w_r: jax.Array,
    B_w_gate: jax.Array,
    B_w_up: jax.Array,
    B_w_down: jax.Array,
):
    del B_x
    kT = jnp.swapaxes(A_k_cache, 2, 3).reshape(B, HD, S)
    vT = jnp.swapaxes(A_v_cache, 2, 3).reshape(B, HD, S)
    x = A_x.reshape(B, D)
    wr = B_w_r.reshape(1, D)
    any_spec = pl.BlockSpec(memory_space=pl.ANY)
    vmem_spec = pl.BlockSpec(memory_space=pltpu.VMEM)
    out = pl.pallas_call(
        _kernel,
        in_specs=[vmem_spec, vmem_spec] + [any_spec] * 7,
        out_specs=vmem_spec,
        out_shape=jax.ShapeDtypeStruct((B, D), A_x.dtype),
        scratch_shapes=[
            pltpu.VMEM((B, NJ, HD, LANES), bf16),
            pltpu.VMEM((B, NJ, HD, LANES), bf16),
            pltpu.VMEM((NC, D, LANES), bf16),
            pltpu.VMEM((ND, HD, LANES), bf16),
            pltpu.VMEM((NF, D, LANES), bf16),
            pltpu.VMEM((NF, D, LANES), bf16),
            pltpu.VMEM((ND, F, LANES), bf16),
            pltpu.VMEM((B, D), f32),
            pltpu.VMEM((B, D), f32),
            pltpu.SemaphoreType.DMA((5,)),
            pltpu.SemaphoreType.DMA((B,)),
            pltpu.SemaphoreType.DMA((B, len(V_PIECES))),
        ],
        compiler_params=pltpu.CompilerParams(vmem_limit_bytes=126 * 1024 * 1024),
    )(x, wr, kT, vT, A_wq, A_wo, B_w_gate, B_w_up, B_w_down)
    return out.reshape(A_x.shape)
```

```python
import functools

import jax
import jax.numpy as jnp
import numpy as np
from jax import lax
from jax.experimental import pallas as pl
from jax.experimental.pallas import tpu as pltpu

B, D, H, DH, S, F = 4, 640, 32, 192, 4096, 1536
W = min(4096, max(256, S // 4))
HD = H * DH
LANES = 128
NJ = W // LANES
NC = HD // LANES
ND = D // LANES
NF = F // LANES
EPS = 1e-5
SCALE = DH ** -0.5

G = 16
NG = H // G
CPG = G * DH // LANES
V_PIECES = (7, 4, 3, 2)
assert sum(V_PIECES) * 3 == NC

bf16 = jnp.bfloat16
f32 = jnp.float32


def _nn(a, b):
    return jnp.dot(a, b, preferred_element_type=f32)


def _nt(a, b):
    return lax.dot_general(a, b, (((1,), (1,)), ((), ())), preferred_element_type=f32)


def _layernorm(xs):
    tot = functools.reduce(jnp.add, xs)
    mean = jnp.sum(tot, axis=1, keepdims=True) * (1.0 / D)
    cs = [x - mean for x in xs]
    sq = functools.reduce(jnp.add, [c * c for c in cs])
    var = jnp.sum(sq, axis=1, keepdims=True) * (1.0 / D)
    inv = lax.rsqrt(var + EPS)
    return [c * inv for c in cs]


def _kernel(x_ref, wr_ref, kT, vT, wq_h, wo_h, wg_h, wu_h, wd_h, o_ref,
            kbuf, vbuf, wq, wo, wg, wu, wd, xs_ref, ys_ref, qbd, obd, wsem, ksem, vsem):

    def col(j):
        return pl.ds(pl.multiple_of(S - W + LANES * j, LANES), LANES)

    def loop(n, fn):
        lax.fori_loop(0, n, lambda i, c: (fn(i), c)[1], 0)

    def start_k(b):
        loop(NJ, lambda j: pltpu.make_async_copy(kT.at[b, :, col(j)], kbuf.at[b, j], ksem.at[b]).start())

    def wait_k(b):
        pltpu.make_async_copy(kbuf.at[b], kbuf.at[b], ksem.at[b]).wait()

    def piece_rows(p):
        return pl.ds(3 * sum(V_PIECES[:p]) * LANES, 3 * V_PIECES[p] * LANES)

    def start_v_whole(b):
        loop(NJ, lambda j: pltpu.make_async_copy(vT.at[b, :, col(j)], vbuf.at[b, j], vsem.at[b, 0]).start())

    def wait_v_whole(b):
        pltpu.make_async_copy(vbuf.at[b], vbuf.at[b], vsem.at[b, 0]).wait()

    def start_v_piece(b, p):
        rows = piece_rows(p)
        loop(NJ, lambda j: pltpu.make_async_copy(
            vT.at[b, rows, col(j)], vbuf.at[b, j, rows], vsem.at[b, p]).start())

    def wait_v_piece(b, p):
        dst = vbuf.at[b, :, piece_rows(p)]
        pltpu.make_async_copy(dst, dst, vsem.at[b, p]).wait()

    def start_w(src, dst, n, sem):
        loop(n, lambda c: pltpu.make_async_copy(
            src.at[:, pl.ds(pl.multiple_of(LANES * c, LANES), LANES)], dst.at[c], sem).start())

    def wait_w(dst, sem):
        pltpu.make_async_copy(dst, dst, sem).wait()

    start_w(wq_h, wq, NC, wsem.at[0])
    start_k(0)

    xs_ref[...] = x_ref[...].astype(f32)
    wr = wr_ref[...].astype(f32)
    wr_t = [jnp.broadcast_to(wr[:, LANES * n:LANES * (n + 1)], (G, LANES)) for n in range(ND)]

    row = lax.broadcasted_iota(jnp.int32, (G, LANES), 0)
    lane = lax.broadcasted_iota(jnp.int32, (G, LANES), 1)

    def head_mask(c):
        col = lane + c * LANES
        lo = row * DH
        return (col >= lo) & (col < lo + DH)

    wait_w(wq, wsem.at[0])
    start_v_whole(0)
    start_w(wo_h, wo, ND, wsem.at[1])
    start_w(wg_h, wg, NF, wsem.at[2])
    start_w(wu_h, wu, NF, wsem.at[3])
    start_w(wd_h, wd, ND, wsem.at[4])

    v_first_tile = {3 * sum(V_PIECES[:p]): p for p in range(len(V_PIECES))}

    def layer(b, xs, first):
        xn = [t.astype(bf16) for t in _layernorm(xs)]
        xnb = jnp.concatenate(xn, axis=1)
        if first:
            wait_k(b)

            @pl.when(b + 1 < B)
            def _():
                start_k(b + 1)

            @pl.when(b + 2 < B)
            def _():
                start_v_whole(b + 1)

            @pl.when(b + 2 == B)
            def _():
                for p in range(len(V_PIECES)):
                    start_v_piece(b + 1, p)

        for cc in range(NC):
            qt = _nn(xnb, wq[cc])
            qbd[cc] = jnp.where(head_mask(cc % CPG), qt, 0.0).astype(bf16)
        acc_o = [None] * ND
        for g in range(NG):
            sc = [None] * NJ
            for c in range(CPG):
                cc = g * CPG + c
                qt = qbd[cc]
                for j in range(NJ):
                    t = _nn(qt, kbuf[b, j, pl.ds(cc * LANES, LANES), :])
                    sc[j] = t if sc[j] is None else sc[j] + t
            m = functools.reduce(jnp.maximum, sc)
            m = jnp.max(m, axis=1, keepdims=True)
            es = [jnp.exp((t - m) * SCALE) for t in sc]
            l = jnp.sum(functools.reduce(jnp.add, es), axis=1, keepdims=True)
            inv = 1.0 / l
            ps = [(e * inv).astype(bf16) for e in es]
            for c in range(CPG):
                cc = g * CPG + c
                if first and cc in v_first_tile:
                    p = v_first_tile[cc]

                    @pl.when(b == B - 1)
                    def _():
                        wait_v_piece(b, p)

                    if cc == 0:
                        @pl.when(b < B - 1)
                        def _():
                            wait_v_whole(b)

                        @pl.when(b == 0)
                        def _():
                            wait_w(wo, wsem.at[1])
                ot = None
                for j in range(NJ):
                    t = _nt(ps[j], vbuf[b, j, pl.ds(cc * LANES, LANES), :])
                    ot = t if ot is None else ot + t
                obd[cc] = jnp.where(head_mask(c), ot, 0.0).astype(bf16)
        for cc in range(NC):
            ot = obd[cc]
            for n in range(ND):
                t = _nn(ot, wo[n, pl.ds(cc * LANES, LANES), :])
                acc_o[n] = t if acc_o[n] is None else acc_o[n] + t
        x1 = [x + jnp.sum(a, axis=0, keepdims=True) for x, a in zip(xs, acc_o)]

        if first:
            @pl.when(b == 0)
            def _():
                wait_w(wg, wsem.at[2])
                wait_w(wu, wsem.at[3])
                wait_w(wd, wsem.at[4])
        xn = _layernorm(x1)
        xnb_t = [t.astype(bf16) for t in xn]
        xnb = jnp.concatenate(xnb_t, axis=1)
        rr = functools.reduce(jnp.add, [a.astype(f32) * w for a, w in zip(xnb_t, wr_t)])
        r = jnp.sum(rr, axis=1, keepdims=True)
        gate = jax.nn.sigmoid(r)
        y = [None] * ND
        for f in range(NF):
            gt = _nn(xnb, wg[f])
            ut = _nn(xnb, wu[f])
            h = (gt * jax.nn.sigmoid(gt) * ut).astype(bf16)
            for n in range(ND):
                t = _nn(h, wd[n, pl.ds(f * LANES, LANES), :])
                y[n] = t if y[n] is None else y[n] + t
        return [a + bb + c * gate for a, bb, c in zip(x1, xn, y)]

    def batch(b, carry):
        x = jnp.broadcast_to(xs_ref[pl.ds(b, 1), :], (G, D))
        xs = [x[:, LANES * n:LANES * (n + 1)] for n in range(ND)]
        xs = layer(b, xs, True)
        xs = layer(b, xs, False)
        ys_ref[pl.ds(b, 1), :] = jnp.concatenate(xs, axis=1)[0:1, :]
        return carry

    lax.fori_loop(0, B, batch, 0)
    o_ref[...] = ys_ref[...].astype(o_ref.dtype)


@jax.jit
def pallas_interleave_layers__sliding_block_cached__moe_arch_mod__decode_kernel(
    A_x: jax.Array,
    A_k_cache: jax.Array,
    A_v_cache: jax.Array,
    A_wq: jax.Array,
    A_wo: jax.Array,
    B_x: jax.Array,
    B_w_r: jax.Array,
    B_w_gate: jax.Array,
    B_w_up: jax.Array,
    B_w_down: jax.Array,
):
    del B_x
    kT = jnp.swapaxes(A_k_cache, 2, 3).reshape(B, HD, S)
    vT = jnp.swapaxes(A_v_cache, 2, 3).reshape(B, HD, S)
    x = A_x.reshape(B, D)
    wr = B_w_r.reshape(1, D)
    any_spec = pl.BlockSpec(memory_space=pl.ANY)
    vmem_spec = pl.BlockSpec(memory_space=pltpu.VMEM)
    out = pl.pallas_call(
        _kernel,
        in_specs=[vmem_spec, vmem_spec] + [any_spec] * 7,
        out_specs=vmem_spec,
        out_shape=jax.ShapeDtypeStruct((B, D), A_x.dtype),
        scratch_shapes=[
            pltpu.VMEM((B, NJ, HD, LANES), bf16),
            pltpu.VMEM((B, NJ, HD, LANES), bf16),
            pltpu.VMEM((NC, D, LANES), bf16),
            pltpu.VMEM((ND, HD, LANES), bf16),
            pltpu.VMEM((NF, D, LANES), bf16),
            pltpu.VMEM((NF, D, LANES), bf16),
            pltpu.VMEM((ND, F, LANES), bf16),
            pltpu.VMEM((B, D), f32),
            pltpu.VMEM((B, D), f32),
            pltpu.VMEM((NC, G, LANES), bf16),
            pltpu.VMEM((NC, G, LANES), bf16),
            pltpu.SemaphoreType.DMA((5,)),
            pltpu.SemaphoreType.DMA((B,)),
            pltpu.SemaphoreType.DMA((B, len(V_PIECES))),
        ],
        compiler_params=pltpu.CompilerParams(vmem_limit_bytes=126 * 1024 * 1024),
    )(x, wr, kT, vT, A_wq, A_wo, B_w_gate, B_w_up, B_w_down)
    return out.reshape(A_x.shape)
```

```python
import functools

import jax
import jax.numpy as jnp
from jax import lax
from jax.experimental import pallas as pl
from jax.experimental.pallas import tpu as pltpu

B, D, H, DH, S, F = 4, 640, 32, 192, 4096, 1536
W = min(4096, max(256, S // 4))
HD = H * DH
LANES = 128
NJ = W // LANES
NC = HD // LANES
ND = D // LANES
NF = F // LANES
EPS = 1e-5
SCALE = DH ** -0.5

G = 16
NG = H // G
CPG = G * DH // LANES
V_PIECES = (7, 4, 3, 2)
assert sum(V_PIECES) * 3 == NC
PIECE_T0 = [3 * sum(V_PIECES[:p]) for p in range(len(V_PIECES) + 1)]

L2_GROUPS = ((0, 4, 'v'), (4, 8, 'v'), (12, 12, 'm'), (24, 8, 'v'))
assert sum(n for _, n, _ in L2_GROUPS) == H

bf16 = jnp.bfloat16
u32 = jnp.uint32
f32 = jnp.float32


def _nn(a, b):
    return jnp.dot(a, b, preferred_element_type=f32)


def _nt(a, b):
    return lax.dot_general(a, b, (((1,), (1,)), ((), ())), preferred_element_type=f32)


def _acc(a, t):
    return t if a is None else a + t


def _layernorm(xs):
    tot = functools.reduce(jnp.add, xs)
    mean = jnp.sum(tot, axis=1, keepdims=True) * (1.0 / D)
    cs = [x - mean for x in xs]
    sq = functools.reduce(jnp.add, [c * c for c in cs])
    var = jnp.sum(sq, axis=1, keepdims=True) * (1.0 / D)
    inv = lax.rsqrt(var + EPS)
    return [c * inv for c in cs]


def _tile(c):
    return pl.ds(c * (LANES // 2), LANES // 2)


def _unpack(w):
    lo = pltpu.bitcast(w << 16, f32)
    hi = pltpu.bitcast(w & jnp.uint32(0xFFFF0000), f32)
    return lo, hi


def _kernel(x_h, wr_h, kT, vT, wq_h, wo_h, wg_h, wu_h, wd_h, o_ref,
            kbuf, vbuf, wq, wo, wg, wu, wd, x_v, wr_v, xs_ref, ys_ref, q1, qbd, obd, hbuf,
            wsem, ksem, vsem):

    k32, v32, wq32, wo32, wg32, wu32, wd32 = (
        r.bitcast(u32) for r in (kbuf, vbuf, wq, wo, wg, wu, wd))

    def ld(ref32, *idx):
        return pltpu.bitcast(ref32[idx], bf16)

    def col(j):
        return pl.ds(pl.multiple_of(S - W + LANES * j, LANES), LANES)

    def loop(n, fn):
        lax.fori_loop(0, n, lambda i, c: (fn(i), c)[1], 0)

    def start_k(b):
        loop(NJ, lambda j: pltpu.make_async_copy(kT.at[b, :, col(j)], kbuf.at[b, j], ksem.at[b]).start())

    def wait_k(b):
        pltpu.make_async_copy(kbuf.at[b], kbuf.at[b], ksem.at[b]).wait()

    def piece_rows(p):
        return pl.ds(PIECE_T0[p] * LANES, (PIECE_T0[p + 1] - PIECE_T0[p]) * LANES)

    def start_v_whole(b):
        loop(NJ, lambda j: pltpu.make_async_copy(vT.at[b, :, col(j)], vbuf.at[b, j], vsem.at[b, 0]).start())

    def wait_v_whole(b):
        pltpu.make_async_copy(vbuf.at[b], vbuf.at[b], vsem.at[b, 0]).wait()

    def start_v_piece(b, p):
        rows = piece_rows(p)
        loop(NJ, lambda j: pltpu.make_async_copy(
            vT.at[b, rows, col(j)], vbuf.at[b, j, rows], vsem.at[b, p]).start())

    def wait_v_piece(b, p):
        dst = vbuf.at[b, :, piece_rows(p)]
        pltpu.make_async_copy(dst, dst, vsem.at[b, p]).wait()

    def start_w(src, dst, n, sem):
        loop(n, lambda c: pltpu.make_async_copy(
            src.at[:, pl.ds(pl.multiple_of(LANES * c, LANES), LANES)], dst.at[c], sem).start())

    def wait_w(dst, sem):
        pltpu.make_async_copy(dst, dst, sem).wait()

    x_cp = pltpu.make_async_copy(x_h, x_v, wsem.at[5])
    wr_cp = pltpu.make_async_copy(wr_h, wr_v, wsem.at[6])

    start_w(wq_h, wq, NC, wsem.at[0])
    x_cp.start()
    wr_cp.start()
    start_k(0)
    x_cp.wait()
    wr_cp.wait()

    xs_ref[...] = x_v[...].astype(f32)
    wr = wr_v[...].astype(f32).reshape(1, D)
    wr_t = [jnp.broadcast_to(wr[:, LANES * n:LANES * (n + 1)], (G, LANES)) for n in range(ND)]

    row = lax.broadcasted_iota(jnp.int32, (G, LANES), 0)
    lane = lax.broadcasted_iota(jnp.int32, (G, LANES), 1)

    def head_mask(c):
        colm = lane + c * LANES
        lo = row * DH
        return (colm >= lo) & (colm < lo + DH)

    wait_w(wq, wsem.at[0])
    start_v_whole(0)
    start_w(wo_h, wo, ND, wsem.at[1])
    start_w(wg_h, wg, NF, wsem.at[2])
    start_w(wu_h, wu, NF, wsem.at[3])
    start_w(wd_h, wd, ND, wsem.at[4])

    def q_phase(xs):
        xn = [t.astype(bf16) for t in _layernorm(xs)]
        xnb = jnp.concatenate(xn, axis=1)
        for cc in range(NC):
            qt = _nn(xnb, ld(wq32, cc))
            qbd[cc] = jnp.where(head_mask(cc % CPG), qt, 0.0).astype(bf16)

    def qk_softmax(b, g):
        sc = [None] * NJ
        for c in range(CPG):
            cc = g * CPG + c
            qt = qbd[cc]
            for j in range(NJ):
                sc[j] = _acc(sc[j], _nn(qt, ld(k32, b, j, _tile(cc), slice(None))))
        m = functools.reduce(jnp.maximum, sc)
        m = jnp.max(m, axis=1, keepdims=True)
        es = [jnp.exp((t - m) * SCALE) for t in sc]
        l = jnp.sum(functools.reduce(jnp.add, es), axis=1, keepdims=True)
        inv = 1.0 / l
        return [(e * inv).astype(bf16) for e in es]

    def pv(b, ps, t0, t1):
        for cc in range(t0, t1):
            g, c = divmod(cc, CPG)
            ot = None
            for j in range(NJ):
                ot = _acc(ot, _nt(ps[g][j], ld(v32, b, j, _tile(cc), slice(None))))
            obd[cc] = jnp.where(head_mask(c), ot, 0.0).astype(bf16)

    def wo_phase(acc_o, t0, t1):
        acc_o = list(acc_o)
        for cc in range(t0, t1):
            ot = obd[cc]
            for n in range(ND):
                acc_o[n] = _acc(acc_o[n], _nn(ot, ld(wo32, n, _tile(cc), slice(None))))
        return acc_o

    def ffn(x1):
        xn = _layernorm(x1)
        xnb_t = [t.astype(bf16) for t in xn]
        xnb = jnp.concatenate(xnb_t, axis=1)
        rr = functools.reduce(jnp.add, [a.astype(f32) * w for a, w in zip(xnb_t, wr_t)])
        gate = jax.nn.sigmoid(jnp.sum(rr, axis=1, keepdims=True))
        for f in range(NF):
            gt = _nn(xnb, ld(wg32, f))
            ut = _nn(xnb, ld(wu32, f))
            hbuf[f] = (gt * jax.nn.sigmoid(gt) * ut).astype(bf16)
        y = [None] * ND
        for f in range(NF):
            h = hbuf[f]
            for n in range(ND):
                y[n] = _acc(y[n], _nn(h, ld(wd32, n, _tile(f), slice(None))))
        return [a + bb + c * gate for a, bb, c in zip(x1, xn, y)]

    def q_phase2(xs):
        xn = [t.astype(bf16) for t in _layernorm(xs)]
        xnb = jnp.concatenate(xn, axis=1)
        for h0, nh, _ in L2_GROUPS:
            for c in range(nh * DH // LANES):
                cc = h0 * DH // LANES + c
                qt = _nn(xnb, ld(wq32, cc))
                qbd[cc] = jnp.where(head_mask(c), qt, 0.0).astype(bf16)

    def attention2(b):
        st = {}
        mxu, vpu = [], []

        def qk_step(gi, cc, j):
            def fn():
                nh = L2_GROUPS[gi][1]
                t = _nn(qbd[cc], ld(k32, b, j, _tile(cc), slice(None)))
                if nh <= 8:
                    t = t[:8]
                st['sc', gi, j] = _acc(st.get(('sc', gi, j)), t)
            return fn

        def sm_step(gi):
            def fn():
                sc = [st['sc', gi, j] for j in range(NJ)]
                m = jnp.max(functools.reduce(jnp.maximum, sc), axis=1, keepdims=True)
                es = [jnp.exp((t - m) * SCALE) for t in sc]
                l = jnp.sum(functools.reduce(jnp.add, es), axis=1, keepdims=True)
                inv = 1.0 / l
                ps = [e * inv for e in es]
                if L2_GROUPS[gi][2] == 'm':
                    ps = [p.astype(bf16) for p in ps]
                st['p', gi] = ps
            return fn

        def vpv_step(gi, r, rg):
            def fn():
                h0 = L2_GROUPS[gi][0]
                if rg == 0:
                    st['pb'] = [jnp.broadcast_to(p[r:r + 1, :], (8, LANES)) for p in st['p', gi]]
                w0 = ((h0 + r) * DH) // 2 + rg * 8
                lo = hi = None
                for j in range(NJ):
                    a, c_ = _unpack(v32[b, j, pl.ds(w0, 8), :])
                    lo = _acc(lo, a * st['pb'][j])
                    hi = _acc(hi, c_ * st['pb'][j])
                st['o', gi, r, rg] = (jnp.sum(lo, axis=1, keepdims=True),
                                      jnp.sum(hi, axis=1, keepdims=True))
            return fn

        def vwo_step(gi, r, rg):
            def fn():
                h0 = L2_GROUPS[gi][0]
                w0 = ((h0 + r) * DH) // 2 + rg * 8
                olo, ohi = st.pop(('o', gi, r, rg))
                for n in range(ND):
                    a, c_ = _unpack(wo32[n, pl.ds(w0, 8), :])
                    st['vacc', n] = _acc(st.get(('vacc', n)), a * olo + c_ * ohi)
            return fn

        def pv_step(gi, cc, c, j):
            def fn():
                p = st['p', gi][j]
                if p.shape[0] == 8:
                    p = jnp.concatenate([p, jnp.zeros_like(p)], axis=0)
                t = _nt(p, ld(v32, b, j, _tile(cc), slice(None)))
                st['ot', cc] = _acc(st.get(('ot', cc)), t)
                if j == NJ - 1:
                    st['ot', cc] = jnp.where(head_mask(c), st['ot', cc], 0.0).astype(bf16)
            return fn

        def wo_step(cc, n):
            def fn():
                st['macc', n] = _acc(st.get(('macc', n)),
                                     _nn(st['ot', cc], ld(wo32, n, _tile(cc), slice(None))))
            return fn

        for gi, (h0, nh, unit) in enumerate(L2_GROUPS):
            c0 = h0 * DH // LANES
            for c in range(nh * DH // LANES):
                for j in range(NJ):
                    mxu.append((8, None, ('qk', gi), qk_step(gi, c0 + c, j)))
        for gi, (h0, nh, unit) in enumerate(L2_GROUPS):
            vpu.append((60 + 6 * nh, ('qk', gi), ('sm', gi), sm_step(gi)))
            if unit == 'v':
                seq = [(r, rg) for r in range(nh) for rg in range(DH // 16)]
                for i, (r, rg) in enumerate(seq):
                    vpu.append((13.5, None, None, vpv_step(gi, r, rg)))
                    if i > 0:
                        vpu.append((8.5, None, None, vwo_step(gi, *seq[i - 1])))
                vpu.append((8.5, None, None, vwo_step(gi, *seq[-1])))
            else:
                c0 = h0 * DH // LANES
                nt = nh * DH // LANES
                for c in range(nt + 1):
                    if c < nt:
                        for j in range(NJ):
                            mxu.append((16, ('sm', gi), None, pv_step(gi, c0 + c, c, j)))
                    if c > 0:
                        for n in range(ND):
                            mxu.append((8, None, None, wo_step(c0 + c - 1, n)))
        order_sm = [i for i, s_ in enumerate(vpu) if s_[1] is not None]

        done = {}
        remaining = {}
        for s_ in mxu + vpu:
            if s_[2] is not None:
                remaining[s_[2]] = remaining.get(s_[2], 0) + 1
        tm = tv = 0.0
        im = 0
        pend = list(vpu)
        LAT = 90.0

        def ready(s_):
            return s_[1] is None or s_[1] in done

        while im < len(mxu) or pend:
            cand = None
            for k_, s_ in enumerate(pend):
                if s_[1] is not None and s_[1] in done:
                    cand = k_
                    break
            if cand is None and pend and ready(pend[0]):
                cand = 0
            m_ok = im < len(mxu) and ready(mxu[im])
            if cand is not None and (not m_ok or tv <= tm):
                cost, dep, tag, fn = pend.pop(cand)
                if dep is not None:
                    tv = max(tv, done[dep] + LAT)
                fn()
                tv += cost
                t_end = tv
            elif m_ok:
                cost, dep, tag, fn = mxu[im]
                im += 1
                if dep is not None:
                    tm = max(tm, done[dep] + LAT)
                fn()
                tm += cost
                t_end = tm
            else:
                raise RuntimeError('schedule deadlock')
            if tag is not None:
                remaining[tag] -= 1
                if remaining[tag] == 0:
                    done[tag] = t_end
        out = []
        for n in range(ND):
            tot = None
            if ('macc', n) in st:
                tot = jnp.sum(st['macc', n], axis=0, keepdims=True)
            if ('vacc', n) in st:
                t = jnp.sum(st['vacc', n], axis=0, keepdims=True)
                tot = t if tot is None else tot + t
            out.append(tot)
        return out

    def layer2(b, xs):
        q_phase2(xs)
        attn = attention2(b)
        return ffn([x + a for x, a in zip(xs, attn)])

    def layer(b, xs, first):
        q_phase(xs)
        if first:
            wait_k(b)

            @pl.when(b + 1 < B)
            def _():
                start_k(b + 1)

            @pl.when(b + 2 < B)
            def _():
                start_v_whole(b + 1)

            @pl.when(b + 2 == B)
            def _():
                for p in range(len(V_PIECES)):
                    start_v_piece(b + 1, p)

        ps = [qk_softmax(b, g) for g in range(NG)]
        acc_o = [None] * ND
        npc = len(V_PIECES)
        if first:
            @pl.when(b < B - 1)
            def _():
                wait_v_whole(b)

            @pl.when(b == 0)
            def _():
                wait_w(wo, wsem.at[1])

            for p in range(npc):
                @pl.when(b == B - 1)
                def _():
                    wait_v_piece(b, p)

                pv(b, ps, PIECE_T0[p], PIECE_T0[p + 1])
                if p > 0:
                    acc_o = wo_phase(acc_o, PIECE_T0[p - 1], PIECE_T0[p])
            acc_o = wo_phase(acc_o, PIECE_T0[npc - 1], NC)
        else:
            pv(b, ps, 0, NC)
            acc_o = wo_phase(acc_o, 0, NC)
        x1 = [x + jnp.sum(a, axis=0, keepdims=True) for x, a in zip(xs, acc_o)]
        if first:
            @pl.when(b == 0)
            def _():
                wait_w(wg, wsem.at[2])
                wait_w(wu, wsem.at[3])
                wait_w(wd, wsem.at[4])
        return ffn(x1)

    def batch(b, carry):
        x = jnp.broadcast_to(xs_ref[pl.ds(b, 1), :], (G, D))
        xs = [x[:, LANES * n:LANES * (n + 1)] for n in range(ND)]
        xs = layer(b, xs, True)
        xs = layer2(b, xs)
        ys_ref[pl.ds(b, 1), :] = jnp.concatenate(xs, axis=1)[0:1, :]
        return carry

    lax.fori_loop(0, B, batch, 0)
    o_ref[...] = ys_ref[...].astype(o_ref.dtype)


@jax.jit
def pallas_interleave_layers__sliding_block_cached__moe_arch_mod__decode_kernel(
    A_x: jax.Array,
    A_k_cache: jax.Array,
    A_v_cache: jax.Array,
    A_wq: jax.Array,
    A_wo: jax.Array,
    B_x: jax.Array,
    B_w_r: jax.Array,
    B_w_gate: jax.Array,
    B_w_up: jax.Array,
    B_w_down: jax.Array,
):
    del B_x
    kT = jnp.swapaxes(A_k_cache, 2, 3).reshape(B, HD, S)
    vT = jnp.swapaxes(A_v_cache, 2, 3).reshape(B, HD, S)
    x = A_x.reshape(B, D)
    any_spec = pl.BlockSpec(memory_space=pl.ANY)
    out = pl.pallas_call(
        _kernel,
        in_specs=[any_spec] * 9,
        out_specs=pl.BlockSpec(memory_space=pltpu.VMEM),
        out_shape=jax.ShapeDtypeStruct((B, D), A_x.dtype),
        scratch_shapes=[
            pltpu.VMEM((B, NJ, HD, LANES), bf16),
            pltpu.VMEM((B, NJ, HD, LANES), bf16),
            pltpu.VMEM((NC, D, LANES), bf16),
            pltpu.VMEM((ND, HD, LANES), bf16),
            pltpu.VMEM((NF, D, LANES), bf16),
            pltpu.VMEM((NF, D, LANES), bf16),
            pltpu.VMEM((ND, F, LANES), bf16),
            pltpu.VMEM((B, D), bf16),
            pltpu.VMEM((D,), bf16),
            pltpu.VMEM((B, D), f32),
            pltpu.VMEM((B, D), f32),
            pltpu.VMEM((NC, 8, LANES), f32),
            pltpu.VMEM((NC, G, LANES), bf16),
            pltpu.VMEM((NC, G, LANES), bf16),
            pltpu.VMEM((NF, G, LANES), bf16),
            pltpu.SemaphoreType.DMA((7,)),
            pltpu.SemaphoreType.DMA((B,)),
            pltpu.SemaphoreType.DMA((B, len(V_PIECES))),
        ],
        compiler_params=pltpu.CompilerParams(vmem_limit_bytes=126 * 1024 * 1024),
    )(x, B_w_r, kT, vT, A_wq, A_wo, B_w_gate, B_w_up, B_w_down)
    return out.reshape(A_x.shape)
```

```python
import functools

import jax
import jax.numpy as jnp
from jax import lax
from jax.experimental import pallas as pl
from jax.experimental.pallas import tpu as pltpu

B, D, H, DH, S, F = 4, 640, 32, 192, 4096, 1536
W = min(4096, max(256, S // 4))
HD = H * DH
LANES = 128
NJ = W // LANES
NC = HD // LANES
ND = D // LANES
NF = F // LANES
EPS = 1e-5
SCALE = DH ** -0.5

G = 16
NG = H // G
CPG = G * DH // LANES
V_PIECES = (8, 4, 2, 1, 1)
assert sum(V_PIECES) * 3 == NC
PIECE_T0 = [3 * sum(V_PIECES[:p]) for p in range(len(V_PIECES) + 1)]

L2_GROUPS = ((0, 2), (2, 6), (8, 8), (16, 8), (24, 8))
assert sum(n for _, n in L2_GROUPS) == H
SM_COST, PV_COST, DEP_LAT, K_AHEAD, SM_POS = 90.0, 12.5, 90.0, 2, 0.5

WPAD = 0
PAD = 0

FLAGS = None
DBG = ()
WO_BLOCKS = 8
WD_BLOCKS = 2
KORDER = 'j'

bf16 = jnp.bfloat16
u32 = jnp.uint32
f32 = jnp.float32


def _nn(a, b):
    return jnp.dot(a, b, preferred_element_type=f32)


def _nt(a, b):
    return lax.dot_general(a, b, (((1,), (1,)), ((), ())), preferred_element_type=f32)


def _acc(a, t):
    return t if a is None else a + t


def _layernorm(xs):
    tot = functools.reduce(jnp.add, xs)
    mean = jnp.sum(tot, axis=1, keepdims=True) * (1.0 / D)
    cs = [x - mean for x in xs]
    sq = functools.reduce(jnp.add, [c * c for c in cs])
    var = jnp.sum(sq, axis=1, keepdims=True) * (1.0 / D)
    inv = lax.rsqrt(var + EPS)
    return [c * inv for c in cs]


def _tile(c):
    return pl.ds(c * (LANES // 2), LANES // 2)


def _unpack(w):
    lo = pltpu.bitcast(w << 16, f32)
    hi = pltpu.bitcast(w & jnp.uint32(0xFFFF0000), f32)
    return lo, hi


def _emit(mxu, vpu):
    remaining, done = {}, {}
    for s in mxu + vpu:
        if s[2] is not None:
            remaining[s[2]] = remaining.get(s[2], 0) + 1
    t = [0.0, 0.0]
    idx = [0, 0]
    streams = (mxu, vpu)
    while idx[0] < len(mxu) or idx[1] < len(vpu):
        start = []
        for u in (0, 1):
            if idx[u] >= len(streams[u]):
                start.append(None)
                continue
            dep = streams[u][idx[u]][1]
            if dep is None or dep not in remaining:
                start.append(t[u])
            elif dep in done:
                start.append(max(t[u], done[dep] + DEP_LAT))
            else:
                start.append(None)
        u = min((u for u in (0, 1) if start[u] is not None), key=lambda u: start[u])
        cost, _, tag, fn = streams[u][idx[u]]
        idx[u] += 1
        fn()
        t[u] = start[u] + cost
        if tag is not None:
            remaining[tag] -= 1
            if remaining[tag] == 0:
                done[tag] = t[u]


def _kernel(x_h, wr_h, kT, vT, wq_h, wo_h, wg_h, wu_h, wd_h, o_ref,
            kbuf, vbuf, wq, wo, wg, wu, wd, x_v, wr_v, xs_ref, ys_ref, pbuf, qbd, obd, hbuf,
            wsem, ksem, vsem):

    k32, v32, wq32, wo32, wg32, wu32, wd32 = (
        r.bitcast(u32) for r in (kbuf, vbuf, wq, wo, wg, wu, wd))

    def ld(ref32, *idx):
        return pltpu.bitcast(ref32[idx], bf16)

    def col(j):
        return pl.ds(pl.multiple_of(S - W + LANES * j, LANES), LANES)

    def loop(n, fn):
        lax.fori_loop(0, n, lambda i, c: (fn(i), c)[1], 0)

    def start_k(b):
        loop(NJ, lambda j: pltpu.make_async_copy(kT.at[b, :, col(j)], kbuf.at[b, j, pl.ds(0, HD)], ksem.at[b]).start())

    def wait_k(b):
        dst = kbuf.at[b, :, pl.ds(0, HD)]
        pltpu.make_async_copy(dst, dst, ksem.at[b]).wait()

    def piece_rows(p):
        return pl.ds(PIECE_T0[p] * LANES, (PIECE_T0[p + 1] - PIECE_T0[p]) * LANES)

    def start_v_whole(b):
        loop(NJ, lambda j: pltpu.make_async_copy(vT.at[b, :, col(j)], vbuf.at[b, j, pl.ds(0, HD)], vsem.at[b, 0]).start())

    def wait_v_whole(b):
        dst = vbuf.at[b, :, pl.ds(0, HD)]
        pltpu.make_async_copy(dst, dst, vsem.at[b, 0]).wait()

    def start_v_piece(b, p):
        rows = piece_rows(p)
        loop(NJ, lambda j: pltpu.make_async_copy(
            vT.at[b, rows, col(j)], vbuf.at[b, j, rows], vsem.at[b, p]).start())

    def wait_v_piece(b, p):
        dst = vbuf.at[b, :, piece_rows(p)]
        pltpu.make_async_copy(dst, dst, vsem.at[b, p]).wait()

    def start_w(src, dst, n, sem):
        loop(n, lambda c: pltpu.make_async_copy(
            src.at[:, pl.ds(pl.multiple_of(LANES * c, LANES), LANES)], dst.at[c, pl.ds(0, src.shape[0])], sem).start())

    def start_tall(src, dst, nblk, sem):
        rows = src.shape[0] // nblk

        def fn(i):
            r = pl.ds(pl.multiple_of((i // ND) * rows, 16), rows)
            c = i % ND
            pltpu.make_async_copy(src.at[r, pl.ds(pl.multiple_of(LANES * c, LANES), LANES)],
                                  dst.at[c, r], sem).start()
        loop(nblk * ND, fn)

    def wait_w(dst, rows, sem):
        dst = dst.at[:, pl.ds(0, rows)]
        pltpu.make_async_copy(dst, dst, sem).wait()

    x_cp = pltpu.make_async_copy(x_h, x_v, wsem.at[5])
    wr_cp = pltpu.make_async_copy(wr_h, wr_v, wsem.at[6])

    start_w(wq_h, wq, NC, wsem.at[0])
    x_cp.start()
    wr_cp.start()
    start_k(0)
    x_cp.wait()
    wr_cp.wait()

    xs_ref[...] = x_v[...].astype(f32)
    wr = wr_v[...].astype(f32).reshape(1, D)
    wr_t = [jnp.broadcast_to(wr[:, LANES * n:LANES * (n + 1)], (G, LANES)) for n in range(ND)]

    row = lax.broadcasted_iota(jnp.int32, (G, LANES), 0)
    lane = lax.broadcasted_iota(jnp.int32, (G, LANES), 1)

    def head_mask(c):
        colm = lane + c * LANES
        lo = row * DH
        return (colm >= lo) & (colm < lo + DH)

    wait_w(wq, D, wsem.at[0])
    start_v_whole(0)
    start_tall(wo_h, wo, WO_BLOCKS, wsem.at[1])
    start_w(wg_h, wg, NF, wsem.at[2])
    start_w(wu_h, wu, NF, wsem.at[3])
    start_tall(wd_h, wd, WD_BLOCKS, wsem.at[4])

    def q_phase(xs):
        xn = [t.astype(bf16) for t in _layernorm(xs)]
        xnb = jnp.concatenate(xn, axis=1)
        for cc in range(NC):
            qt = _nn(xnb, ld(wq32, cc, pl.ds(0, D // 2), slice(None)))
            qbd[cc] = jnp.where(head_mask(cc % CPG), qt, 0.0).astype(bf16)

    def qk_softmax(b, g):
        sc = [None] * NJ
        for c in range(CPG):
            cc = g * CPG + c
            qt = qbd[cc]
            for j in range(NJ):
                sc[j] = _acc(sc[j], _nn(qt, ld(k32, b, j, _tile(cc), slice(None))))
        m = functools.reduce(jnp.maximum, sc)
        m = jnp.max(m, axis=1, keepdims=True)
        es = [jnp.exp((t - m) * SCALE) for t in sc]
        l = jnp.sum(functools.reduce(jnp.add, es), axis=1, keepdims=True)
        inv = 1.0 / l
        return [(e * inv).astype(bf16) for e in es]

    def pv(b, ps, t0, t1):
        for cc in range(t0, t1):
            g, c = divmod(cc, CPG)
            ot = None
            for j in range(NJ):
                ot = _acc(ot, _nt(ps[g][j], ld(v32, b, j, _tile(cc), slice(None))))
            obd[cc] = jnp.where(head_mask(c), ot, 0.0).astype(bf16)

    def wo_phase(acc_o, t0, t1):
        acc_o = list(acc_o)
        for cc in range(t0, t1):
            ot = obd[cc]
            for n in range(ND):
                acc_o[n] = _acc(acc_o[n], _nn(ot, ld(wo32, n, _tile(cc), slice(None))))
        return acc_o

    def ffn(x1):
        xn = _layernorm(x1)
        xnb_t = [t.astype(bf16) for t in xn]
        xnb = jnp.concatenate(xnb_t, axis=1)
        rr = functools.reduce(jnp.add, [a.astype(f32) * w for a, w in zip(xnb_t, wr_t)])
        gate = jax.nn.sigmoid(jnp.sum(rr, axis=1, keepdims=True))
        for f in range(NF):
            gt = _nn(xnb, ld(wg32, f, pl.ds(0, D // 2), slice(None)))
            ut = _nn(xnb, ld(wu32, f, pl.ds(0, D // 2), slice(None)))
            hbuf[f] = (gt * jax.nn.sigmoid(gt) * ut).astype(bf16)
        y = [None] * ND
        for f in range(NF):
            h = hbuf[f]
            for n in range(ND):
                y[n] = _acc(y[n], _nn(h, ld(wd32, n, _tile(f), slice(None))))
        return [a + bb + c * gate for a, bb, c in zip(x1, xn, y)]

    def q_phase2(xs):
        xn = [t.astype(bf16) for t in _layernorm(xs)]
        xnb = jnp.concatenate(xn, axis=1)
        for h0, nh in L2_GROUPS:
            for c in range(nh * DH // LANES):
                cc = h0 * DH // LANES + c
                qt = _nn(xnb, ld(wq32, cc, pl.ds(0, D // 2), slice(None)))
                qbd[cc] = jnp.where(head_mask(c), qt, 0.0).astype(bf16)

    sub8 = lax.broadcasted_iota(jnp.int32, (8, LANES), 0)
    lane8 = lax.broadcasted_iota(jnp.int32, (8, LANES), 1)
    diag = lane8 - 2 * sub8

    def attention2(b):
        st = {}
        mxu, vpu = [], []

        def qk_step(gi, cc, j, last):
            def fn():
                if 'nok' in DBG and cc != L2_GROUPS[gi][0] * DH // LANES and not last:
                    return
                t = _nn(qbd[cc], ld(k32, b, j, _tile(cc), slice(None)))[:8]
                t = _acc(st.pop(('sc', gi, j), None), t)
                if last:
                    pbuf[gi, j] = t
                else:
                    st['sc', gi, j] = t
            return fn

        def sm_step(gi):
            def fn():
                sc = [pbuf[gi, j] for j in range(NJ)]
                m = jnp.max(functools.reduce(jnp.maximum, sc), axis=1, keepdims=True)
                es = [jnp.exp((t - m) * SCALE) for t in sc]
                l = jnp.sum(functools.reduce(jnp.add, es), axis=1, keepdims=True)
                inv = 1.0 / l
                for j in range(NJ):
                    pbuf[gi, j] = es[j] * inv
            return fn

        def pv_step(gi, r, rg):
            def fn():
                if rg == 0:
                    st['pb'] = [jnp.broadcast_to(pbuf[gi, j, r:r + 1, :], (8, LANES)) for j in range(NJ)]
                g16 = (L2_GROUPS[gi][0] + r) * (DH // 16) + rg
                cc, k = divmod(g16, LANES // 16)
                lo = hi = None
                for j in range(NJ):
                    a, c_ = _unpack(v32[b, j, pl.ds(g16 * 8, 8), :])
                    lo = _acc(lo, a * st['pb'][j])
                    hi = _acc(hi, c_ * st['pb'][j])
                lo = jnp.sum(lo, axis=1, keepdims=True)
                hi = jnp.sum(hi, axis=1, keepdims=True)
                t = st.get(('ot', cc), jnp.zeros((8, LANES), f32))
                t = jnp.where(diag == 16 * k, lo, t)
                st['ot', cc] = jnp.where(diag == 16 * k + 1, hi, t)
            return fn

        def wo_step(cc, n):
            def fn():
                if 'nowo' in DBG:
                    st['acc', n] = _acc(st.get(('acc', n)), st['ot', cc])
                    return
                if n == 0:
                    st['ot', cc] = st['ot', cc].astype(bf16)
                st['acc', n] = _acc(st.get(('acc', n)),
                                    _nn(st['ot', cc], ld(wo32, n, _tile(cc), slice(None))))
            return fn

        vpu.append((SM_COST, ('qk', 0), None, sm_step(0)))
        for gi, (h0, nh) in enumerate(L2_GROUPS):
            for r in range(nh):
                if r == int(nh * SM_POS) and gi + 1 < len(L2_GROUPS):
                    vpu.append((SM_COST, ('qk', gi + 1), None, sm_step(gi + 1)))
                for rg in range(DH // 16):
                    g16 = (h0 + r) * (DH // 16) + rg
                    vpu.append((PV_COST, None, ('ot', g16 // (LANES // 16)), pv_step(gi, r, rg)))
        def tiles(gi):
            h0, nh = L2_GROUPS[gi]
            return range(h0 * DH // LANES, (h0 + nh) * DH // LANES)
        ng = len(L2_GROUPS)
        for gi in range(ng + K_AHEAD):
            if gi < ng:
                if KORDER == 'j':
                    for j in range(NJ):
                        for cc in tiles(gi):
                            mxu.append((8, None, ('qk', gi), qk_step(gi, cc, j, cc == tiles(gi)[-1])))
                else:
                    for cc in tiles(gi):
                        for j in range(NJ):
                            mxu.append((8, None, ('qk', gi), qk_step(gi, cc, j, cc == tiles(gi)[-1])))
            if gi >= K_AHEAD:
                for cc in tiles(gi - K_AHEAD):
                    for n in range(ND):
                        mxu.append((8, ('ot', cc), None, wo_step(cc, n)))
        _emit(mxu, vpu)
        return [jnp.sum(st['acc', n], axis=0, keepdims=True) for n in range(ND)]

    def layer2(b, xs):
        q_phase2(xs)
        attn = attention2(b)
        return ffn([x + a for x, a in zip(xs, attn)])

    def l1_dma_start(b):
        wait_k(b)

        @pl.when(b + 1 < B)
        def _():
            start_k(b + 1)

        @pl.when(b + 2 < B)
        def _():
            start_v_whole(b + 1)

        @pl.when(b + 2 == B)
        def _():
            for p in range(len(V_PIECES)):
                start_v_piece(b + 1, p)

    def l1_wait_all(b):
        @pl.when(b < B - 1)
        def _():
            wait_v_whole(b)

        for p in range(len(V_PIECES)):
            @pl.when(b == B - 1)
            def _():
                wait_v_piece(b, p)

        @pl.when(b == 0)
        def _():
            wait_w(wo, HD, wsem.at[1])
            wait_w(wg, D, wsem.at[2])
            wait_w(wu, D, wsem.at[3])
            wait_w(wd, F, wsem.at[4])

    def layer(b, xs, first):
        q_phase(xs)
        if first:
            l1_dma_start(b)

        ps = [qk_softmax(b, g) for g in range(NG)]
        acc_o = [None] * ND
        npc = len(V_PIECES)
        if first:
            @pl.when(b < B - 1)
            def _():
                wait_v_whole(b)

            @pl.when(b == 0)
            def _():
                wait_w(wo, HD, wsem.at[1])

            for p in range(npc):
                @pl.when(b == B - 1)
                def _():
                    wait_v_piece(b, p)

                pv(b, ps, PIECE_T0[p], PIECE_T0[p + 1])
                if 0 < p < npc - 1:
                    acc_o = wo_phase(acc_o, PIECE_T0[p - 1], PIECE_T0[p])
                if p >= npc - 2:
                    acc_o = wo_phase(acc_o, PIECE_T0[p], PIECE_T0[p + 1])
        else:
            pv(b, ps, 0, NC)
            acc_o = wo_phase(acc_o, 0, NC)
        x1 = [x + jnp.sum(a, axis=0, keepdims=True) for x, a in zip(xs, acc_o)]
        if first:
            @pl.when(b == 0)
            def _():
                wait_w(wg, D, wsem.at[2])
                wait_w(wu, D, wsem.at[3])
                wait_w(wd, F, wsem.at[4])
        return ffn(x1)

    def batch(b, carry):
        x = jnp.broadcast_to(xs_ref[pl.ds(b, 1), :], (G, D))
        xs = [x[:, LANES * n:LANES * (n + 1)] for n in range(ND)]
        xs = layer(b, xs, True)
        xs = layer2(b, xs)
        ys_ref[pl.ds(b, 1), :] = jnp.concatenate(xs, axis=1)[0:1, :]
        return carry

    lax.fori_loop(0, B, batch, 0)
    o_ref[...] = ys_ref[...].astype(o_ref.dtype)


@jax.jit
def pallas_interleave_layers__sliding_block_cached__moe_arch_mod__decode_kernel(
    A_x: jax.Array,
    A_k_cache: jax.Array,
    A_v_cache: jax.Array,
    A_wq: jax.Array,
    A_wo: jax.Array,
    B_x: jax.Array,
    B_w_r: jax.Array,
    B_w_gate: jax.Array,
    B_w_up: jax.Array,
    B_w_down: jax.Array,
):
    del B_x
    kT = jnp.swapaxes(A_k_cache, 2, 3).reshape(B, HD, S)
    vT = jnp.swapaxes(A_v_cache, 2, 3).reshape(B, HD, S)
    x = A_x.reshape(B, D)
    any_spec = pl.BlockSpec(memory_space=pl.ANY)
    out = pl.pallas_call(
        _kernel,
        in_specs=[any_spec] * 9,
        out_specs=pl.BlockSpec(memory_space=pltpu.VMEM),
        out_shape=jax.ShapeDtypeStruct((B, D), A_x.dtype),
        scratch_shapes=[
            pltpu.VMEM((B, NJ, HD + PAD, LANES), bf16),
            pltpu.VMEM((B, NJ, HD + PAD, LANES), bf16),
            pltpu.VMEM((NC, D + WPAD, LANES), bf16),
            pltpu.VMEM((ND, HD + PAD, LANES), bf16),
            pltpu.VMEM((NF, D + WPAD, LANES), bf16),
            pltpu.VMEM((NF, D + WPAD, LANES), bf16),
            pltpu.VMEM((ND, F + WPAD, LANES), bf16),
            pltpu.VMEM((B, D), bf16),
            pltpu.VMEM((D,), bf16),
            pltpu.VMEM((B, D), f32),
            pltpu.VMEM((B, D), f32),
            pltpu.VMEM((len(L2_GROUPS), NJ, 8, LANES), f32),
            pltpu.VMEM((NC, G, LANES), bf16),
            pltpu.VMEM((NC, G, LANES), bf16),
            pltpu.VMEM((NF, G, LANES), bf16),
            pltpu.SemaphoreType.DMA((7,)),
            pltpu.SemaphoreType.DMA((B,)),
            pltpu.SemaphoreType.DMA((B, len(V_PIECES))),
        ],
        compiler_params=pltpu.CompilerParams(vmem_limit_bytes=126 * 1024 * 1024, flags=FLAGS),
    )(x, B_w_r, kT, vT, A_wq, A_wo, B_w_gate, B_w_up, B_w_down)
    return out.reshape(A_x.shape)
```

```python
import functools

import jax
import jax.numpy as jnp
from jax import lax
from jax.experimental import pallas as pl
from jax.experimental.pallas import tpu as pltpu

B, D, H, DH, S, F = 4, 640, 32, 192, 4096, 1536
W = min(4096, max(256, S // 4))
HD = H * DH
LANES = 128
NJ = W // LANES
NC = HD // LANES
ND = D // LANES
NF = F // LANES
EPS = 1e-5
SCALE = DH ** -0.5

G = 16
NG = H // G
CPG = G * DH // LANES
V_PIECES = (8, 4, 2, 1, 1)
assert sum(V_PIECES) * 3 == NC
PIECE_T0 = [3 * sum(V_PIECES[:p]) for p in range(len(V_PIECES) + 1)]

GROUPS = ((0, 2), (2, 6), (8, 8), (16, 8), (24, 8))
assert sum(n for _, n in GROUPS) == H
SM_COST, DEP_LAT, K_AHEAD, SM_POS = 90.0, 90.0, 2, 0.5
PV_COST = (16.0, 8.5)
EXPAND = True

FLAGS = None
DBG = ()
WO_BLOCKS = 8
WD_BLOCKS = 2
KORDER = 'j'

bf16 = jnp.bfloat16
u32 = jnp.uint32
f32 = jnp.float32


def _nn(a, b):
    return jnp.dot(a, b, preferred_element_type=f32)


def _nt(a, b):
    return lax.dot_general(a, b, (((1,), (1,)), ((), ())), preferred_element_type=f32)


def _acc(a, t):
    return t if a is None else a + t


def _layernorm(xs):
    tot = functools.reduce(jnp.add, xs)
    mean = jnp.sum(tot, axis=1, keepdims=True) * (1.0 / D)
    cs = [x - mean for x in xs]
    sq = functools.reduce(jnp.add, [c * c for c in cs])
    var = jnp.sum(sq, axis=1, keepdims=True) * (1.0 / D)
    inv = lax.rsqrt(var + EPS)
    return [c * inv for c in cs]


def _tile(c):
    return pl.ds(c * (LANES // 2), LANES // 2)


def _unpack(w):
    lo = pltpu.bitcast(w << 16, f32)
    hi = pltpu.bitcast(w & jnp.uint32(0xFFFF0000), f32)
    return lo, hi


def _emit(mxu, vpu):
    remaining, done = {}, {}
    for s in mxu + vpu:
        if s[2] is not None:
            remaining[s[2]] = remaining.get(s[2], 0) + 1
    t = [0.0, 0.0]
    idx = [0, 0]
    streams = (mxu, vpu)
    while idx[0] < len(mxu) or idx[1] < len(vpu):
        start = []
        for u in (0, 1):
            if idx[u] >= len(streams[u]):
                start.append(None)
                continue
            dep = streams[u][idx[u]][1]
            if dep is None or dep not in remaining:
                start.append(t[u])
            elif dep in done:
                start.append(max(t[u], done[dep] + DEP_LAT))
            else:
                start.append(None)
        u = min((u for u in (0, 1) if start[u] is not None), key=lambda u: start[u])
        cost, _, tag, fn = streams[u][idx[u]]
        idx[u] += 1
        fn()
        t[u] = start[u] + cost
        if tag is not None:
            remaining[tag] -= 1
            if remaining[tag] == 0:
                done[tag] = t[u]


def _kernel(x_h, wr_h, kT, vT, wq_h, wo_h, wg_h, wu_h, wd_h, o_ref,
            kbuf, vbuf, wq, wo, wg, wu, wd, x_v, wr_v, xs_ref, ys_ref, pbuf, qbd, hbuf,
            wsem, ksem, vsem):

    k32, v32, wq32, wo32, wg32, wu32, wd32 = (
        r.bitcast(u32) for r in (kbuf, vbuf, wq, wo, wg, wu, wd))

    def ld(ref32, *idx):
        return pltpu.bitcast(ref32[idx], bf16)

    def col(j):
        return pl.ds(pl.multiple_of(S - W + LANES * j, LANES), LANES)

    def loop(n, fn):
        lax.fori_loop(0, n, lambda i, c: (fn(i), c)[1], 0)

    def start_k(b):
        loop(NJ, lambda j: pltpu.make_async_copy(kT.at[b, :, col(j)], kbuf.at[b, j], ksem.at[b]).start())

    def wait_k(b):
        dst = kbuf.at[b]
        pltpu.make_async_copy(dst, dst, ksem.at[b]).wait()

    def piece_rows(p):
        return pl.ds(PIECE_T0[p] * LANES, (PIECE_T0[p + 1] - PIECE_T0[p]) * LANES)

    def start_v_whole(b):
        loop(NJ, lambda j: pltpu.make_async_copy(vT.at[b, :, col(j)], vbuf.at[b, j], vsem.at[b, 0]).start())

    def wait_v_whole(b):
        dst = vbuf.at[b]
        pltpu.make_async_copy(dst, dst, vsem.at[b, 0]).wait()

    def start_v_piece(b, p):
        rows = piece_rows(p)
        loop(NJ, lambda j: pltpu.make_async_copy(
            vT.at[b, rows, col(j)], vbuf.at[b, j, rows], vsem.at[b, p]).start())

    def wait_v_piece(b, p):
        dst = vbuf.at[b, :, piece_rows(p)]
        pltpu.make_async_copy(dst, dst, vsem.at[b, p]).wait()

    def start_w(src, dst, n, sem):
        loop(n, lambda c: pltpu.make_async_copy(
            src.at[:, pl.ds(pl.multiple_of(LANES * c, LANES), LANES)], dst.at[c], sem).start())

    def start_tall(src, dst, nblk, sem):
        rows = src.shape[0] // nblk

        def fn(i):
            r = pl.ds(pl.multiple_of((i // ND) * rows, 16), rows)
            c = i % ND
            pltpu.make_async_copy(src.at[r, pl.ds(pl.multiple_of(LANES * c, LANES), LANES)],
                                  dst.at[c, r], sem).start()
        loop(nblk * ND, fn)

    def wait_w(dst, sem):
        pltpu.make_async_copy(dst, dst, sem).wait()

    x_cp = pltpu.make_async_copy(x_h, x_v, wsem.at[5])
    wr_cp = pltpu.make_async_copy(wr_h, wr_v, wsem.at[6])

    start_w(wq_h, wq, NC, wsem.at[0])
    x_cp.start()
    wr_cp.start()
    start_k(0)
    x_cp.wait()
    wr_cp.wait()

    xs_ref[...] = x_v[...].astype(f32)
    wr = wr_v[...].astype(f32).reshape(1, D)
    wr_t = [jnp.broadcast_to(wr[:, LANES * n:LANES * (n + 1)], (G, LANES)) for n in range(ND)]

    row = lax.broadcasted_iota(jnp.int32, (G, LANES), 0)
    lane = lax.broadcasted_iota(jnp.int32, (G, LANES), 1)

    def head_mask(c):
        colm = lane + c * LANES
        lo = row * DH
        return (colm >= lo) & (colm < lo + DH)

    wait_w(wq, wsem.at[0])
    start_v_whole(0)
    start_tall(wo_h, wo, WO_BLOCKS, wsem.at[1])
    start_w(wg_h, wg, NF, wsem.at[2])
    start_w(wu_h, wu, NF, wsem.at[3])
    start_tall(wd_h, wd, WD_BLOCKS, wsem.at[4])

    def ffn(x1):
        xn = _layernorm(x1)
        xnb_t = [t.astype(bf16) for t in xn]
        xnb = jnp.concatenate(xnb_t, axis=1)
        rr = functools.reduce(jnp.add, [a.astype(f32) * w for a, w in zip(xnb_t, wr_t)])
        gate = jax.nn.sigmoid(jnp.sum(rr, axis=1, keepdims=True))
        for f in range(NF):
            gt = _nn(xnb, ld(wg32, f))
            ut = _nn(xnb, ld(wu32, f))
            hbuf[f] = (gt * jax.nn.sigmoid(gt) * ut).astype(bf16)
        y = [None] * ND
        for f in range(NF):
            h = hbuf[f]
            for n in range(ND):
                y[n] = _acc(y[n], _nn(h, ld(wd32, n, _tile(f), slice(None))))
        return [a + bb + c * gate for a, bb, c in zip(x1, xn, y)]

    sub8 = lax.broadcasted_iota(jnp.int32, (8, LANES), 0)
    lane8 = lax.broadcasted_iota(jnp.int32, (8, LANES), 1)
    diag = lane8 - 2 * sub8

    def tiles(gi):
        h0, nh = GROUPS[gi]
        return range(h0 * DH // LANES, (h0 + nh) * DH // LANES)

    def attention(b, xs, first):
        xlo, xhi = (b + B - 1) % B, (b + B - 2) % B
        xn = [t.astype(bf16) for t in _layernorm(xs)]
        xnb = jnp.concatenate(xn, axis=1)
        for gi in range(len(GROUPS)):
            for c, cc in enumerate(tiles(gi)):
                qt = _nn(xnb, ld(wq32, cc))
                qbd[cc] = jnp.where(head_mask(c), qt, 0.0).astype(bf16)
        if first:
            l1_dma_start(b)

        st = {}
        mxu, vpu = [], []

        def qk_step(gi, cc, j, last):
            def fn():
                t = _nn(qbd[cc], ld(k32, b, j, _tile(cc), slice(None)))[:8]
                t = _acc(st.pop(('sc', gi, j), None), t)
                if last:
                    pbuf[gi, j] = t
                else:
                    st['sc', gi, j] = t
            return fn

        def sm_step(gi):
            def fn():
                sc = [pbuf[gi, j] for j in range(NJ)]
                m = jnp.max(functools.reduce(jnp.maximum, sc), axis=1, keepdims=True)
                es = [jnp.exp((t - m) * SCALE) for t in sc]
                l = jnp.sum(functools.reduce(jnp.add, es), axis=1, keepdims=True)
                inv = 1.0 / l
                for j in range(NJ):
                    pbuf[gi, j] = es[j] * inv
            return fn

        def pv_step(gi, r, rg):
            def fn():
                if rg == 0:
                    st['pb'] = [jnp.broadcast_to(pbuf[gi, j, r:r + 1, :], (8, LANES)) for j in range(NJ)]
                g16 = (GROUPS[gi][0] + r) * (DH // 16) + rg
                cc, k = divmod(g16, LANES // 16)
                rows = pl.ds(g16 * 8, 8)
                lo = hi = None
                for j in range(NJ):
                    if first or not EXPAND:
                        a, c_ = _unpack(v32[b, j, rows, :])
                        if EXPAND:
                            k32[xlo, j, rows, :] = pltpu.bitcast(a, u32)
                            k32[xhi, j, rows, :] = pltpu.bitcast(c_, u32)
                    else:
                        a = pltpu.bitcast(k32[xlo, j, rows, :], f32)
                        c_ = pltpu.bitcast(k32[xhi, j, rows, :], f32)
                    lo = _acc(lo, a * st['pb'][j])
                    hi = _acc(hi, c_ * st['pb'][j])
                lo = jnp.sum(lo, axis=1, keepdims=True)
                hi = jnp.sum(hi, axis=1, keepdims=True)
                t = st.get(('ot', cc), jnp.zeros((8, LANES), f32))
                t = jnp.where(diag == 16 * k, lo, t)
                st['ot', cc] = jnp.where(diag == 16 * k + 1, hi, t)
            return fn

        def wo_step(cc, n):
            def fn():
                if n == 0:
                    st['ot', cc] = st['ot', cc].astype(bf16)
                st['acc', n] = _acc(st.get(('acc', n)),
                                    _nn(st['ot', cc], ld(wo32, n, _tile(cc), slice(None))))
            return fn

        def wait_step(p):
            def fn():
                @pl.when(b == B - 1)
                def _():
                    wait_v_piece(b, p)

                if p == 0:
                    @pl.when(b < B - 1)
                    def _():
                        wait_v_whole(b)

                    @pl.when(b == 0)
                    def _():
                        wait_w(wo, wsem.at[1])
            return fn

        ng = len(GROUPS)
        pv_cost = PV_COST[0 if first else 1]
        if first:
            vpu += [(SM_COST, ('qk', gi), None, sm_step(gi)) for gi in range(ng)]
        else:
            vpu.append((SM_COST, ('qk', 0), None, sm_step(0)))
        for gi, (h0, nh) in enumerate(GROUPS):
            for r in range(nh):
                if not first and r == int(nh * SM_POS) and gi + 1 < ng:
                    vpu.append((SM_COST, ('qk', gi + 1), None, sm_step(gi + 1)))
                for rg in range(DH // 16):
                    g16 = (h0 + r) * (DH // 16) + rg
                    cc, k = divmod(g16, LANES // 16)
                    if first and k == 0 and cc in PIECE_T0[:-1]:
                        vpu.append((0.0, None, None, wait_step(PIECE_T0.index(cc))))
                    vpu.append((pv_cost, None, ('ot', cc), pv_step(gi, r, rg)))
        ahead = ng if first else K_AHEAD
        for gi in range(ng + ahead):
            if gi < ng:
                for cc in tiles(gi):
                    for j in range(NJ):
                        mxu.append((8, None, ('qk', gi), qk_step(gi, cc, j, cc == tiles(gi)[-1])))
            if gi >= ahead:
                for cc in tiles(gi - ahead):
                    for n in range(ND):
                        mxu.append((8, ('ot', cc), None, wo_step(cc, n)))
        _emit(mxu, vpu)
        return [x + jnp.sum(st['acc', n], axis=0, keepdims=True) for n, x in enumerate(xs)]

    def l1_dma_start(b):
        wait_k(b)

        @pl.when(b + 1 < B)
        def _():
            start_k(b + 1)

        @pl.when(b + 2 < B)
        def _():
            start_v_whole(b + 1)

        @pl.when(b + 2 == B)
        def _():
            for p in range(len(V_PIECES)):
                start_v_piece(b + 1, p)

    def l1_wait_all(b):
        @pl.when(b < B - 1)
        def _():
            wait_v_whole(b)

        for p in range(len(V_PIECES)):
            @pl.when(b == B - 1)
            def _():
                wait_v_piece(b, p)

        @pl.when(b == 0)
        def _():
            wait_w(wo, wsem.at[1])
            wait_w(wg, wsem.at[2])
            wait_w(wu, wsem.at[3])
            wait_w(wd, wsem.at[4])

    def layer(b, xs, first):
        x1 = attention(b, xs, first)
        if first:
            @pl.when(b == 0)
            def _():
                wait_w(wg, wsem.at[2])
                wait_w(wu, wsem.at[3])
                wait_w(wd, wsem.at[4])
        return ffn(x1)

    def batch(b, carry):
        x = jnp.broadcast_to(xs_ref[pl.ds(b, 1), :], (G, D))
        xs = [x[:, LANES * n:LANES * (n + 1)] for n in range(ND)]
        xs = layer(b, xs, True)
        xs = layer(b, xs, False)
        ys_ref[pl.ds(b, 1), :] = jnp.concatenate(xs, axis=1)[0:1, :]
        return carry

    lax.fori_loop(0, B, batch, 0)
    o_ref[...] = ys_ref[...].astype(o_ref.dtype)


@jax.jit
def pallas_interleave_layers__sliding_block_cached__moe_arch_mod__decode_kernel(
    A_x: jax.Array,
    A_k_cache: jax.Array,
    A_v_cache: jax.Array,
    A_wq: jax.Array,
    A_wo: jax.Array,
    B_x: jax.Array,
    B_w_r: jax.Array,
    B_w_gate: jax.Array,
    B_w_up: jax.Array,
    B_w_down: jax.Array,
):
    del B_x
    kT = jnp.swapaxes(A_k_cache, 2, 3).reshape(B, HD, S)
    vT = jnp.swapaxes(A_v_cache, 2, 3).reshape(B, HD, S)
    x = A_x.reshape(B, D)
    any_spec = pl.BlockSpec(memory_space=pl.ANY)
    out = pl.pallas_call(
        _kernel,
        in_specs=[any_spec] * 9,
        out_specs=pl.BlockSpec(memory_space=pltpu.VMEM),
        out_shape=jax.ShapeDtypeStruct((B, D), A_x.dtype),
        scratch_shapes=[
            pltpu.VMEM((B, NJ, HD, LANES), bf16),
            pltpu.VMEM((B, NJ, HD, LANES), bf16),
            pltpu.VMEM((NC, D, LANES), bf16),
            pltpu.VMEM((ND, HD, LANES), bf16),
            pltpu.VMEM((NF, D, LANES), bf16),
            pltpu.VMEM((NF, D, LANES), bf16),
            pltpu.VMEM((ND, F, LANES), bf16),
            pltpu.VMEM((B, D), bf16),
            pltpu.VMEM((D,), bf16),
            pltpu.VMEM((B, D), f32),
            pltpu.VMEM((B, D), f32),
            pltpu.VMEM((len(GROUPS), NJ, 8, LANES), f32),
            pltpu.VMEM((NC, G, LANES), bf16),
            pltpu.VMEM((NF, G, LANES), bf16),
            pltpu.SemaphoreType.DMA((7,)),
            pltpu.SemaphoreType.DMA((B,)),
            pltpu.SemaphoreType.DMA((B, len(V_PIECES))),
        ],
        compiler_params=pltpu.CompilerParams(vmem_limit_bytes=126 * 1024 * 1024, flags=FLAGS),
    )(x, B_w_r, kT, vT, A_wq, A_wo, B_w_gate, B_w_up, B_w_down)
    return out.reshape(A_x.shape)
```

```python
import functools

import jax
import jax.numpy as jnp
from jax import lax
from jax.experimental import pallas as pl
from jax.experimental.pallas import tpu as pltpu

B, D, H, DH, S, F = 4, 640, 32, 192, 4096, 1536
W = min(4096, max(256, S // 4))
HD = H * DH
LANES = 128
NJ = W // LANES
NC = HD // LANES
ND = D // LANES
NF = F // LANES
EPS = 1e-5
SCALE = DH ** -0.5

G = 16
NG = H // G
CPG = G * DH // LANES
V_PIECES = (24, 12, 6, 3, 2, 1)
assert sum(V_PIECES) == NC
PIECE_T0 = [sum(V_PIECES[:p]) for p in range(len(V_PIECES) + 1)]

GROUPS = ((0, 2), (2, 6), (8, 8), (16, 8), (24, 8))
assert sum(n for _, n in GROUPS) == H
SM_COST, DEP_LAT, K_AHEAD, SM_POS = 90.0, 90.0, 2, 0.5
PV_COST = (16.0, 8.5)
NX = 8
WV = (1, 7)
QV = tuple(range(2, NC, 3))
QV_BATCH = 2
FV = (3, 7, 11)

FLAGS = None
DBG = ()
WO_BLOCKS = 8
WD_BLOCKS = 2
KORDER = 'j'

bf16 = jnp.bfloat16
u32 = jnp.uint32
f32 = jnp.float32


def _nn(a, b):
    return jnp.dot(a, b, preferred_element_type=f32)


def _nt(a, b):
    return lax.dot_general(a, b, (((1,), (1,)), ((), ())), preferred_element_type=f32)


def _acc(a, t):
    return t if a is None else a + t


def _layernorm(xs):
    s1 = jnp.sum(functools.reduce(jnp.add, xs), axis=1, keepdims=True)
    s2 = jnp.sum(functools.reduce(jnp.add, [x * x for x in xs]), axis=1, keepdims=True)
    mean = s1 * (1.0 / D)
    var = jnp.maximum(s2 * (1.0 / D) - mean * mean, 0.0)
    inv = lax.rsqrt(var + EPS)
    return [(x - mean) * inv for x in xs]


def _tile(c):
    return pl.ds(c * (LANES // 2), LANES // 2)


def _unpack(w):
    lo = pltpu.bitcast(w << 16, f32)
    hi = pltpu.bitcast(w & jnp.uint32(0xFFFF0000), f32)
    return lo, hi


def _emit(mxu, vpu):
    remaining, done = {}, {}
    for s in mxu + vpu:
        if s[2] is not None:
            remaining[s[2]] = remaining.get(s[2], 0) + 1
    t = [0.0, 0.0]
    idx = [0, 0]
    streams = (mxu, vpu)
    while idx[0] < len(mxu) or idx[1] < len(vpu):
        start = []
        for u in (0, 1):
            if idx[u] >= len(streams[u]):
                start.append(None)
                continue
            dep = streams[u][idx[u]][1]
            if dep is None or dep not in remaining:
                start.append(t[u])
            elif dep in done:
                start.append(max(t[u], done[dep] + DEP_LAT))
            else:
                start.append(None)
        u = min((u for u in (0, 1) if start[u] is not None), key=lambda u: start[u])
        cost, _, tag, fn = streams[u][idx[u]]
        idx[u] += 1
        fn()
        t[u] = start[u] + cost
        if tag is not None:
            remaining[tag] -= 1
            if remaining[tag] == 0:
                done[tag] = t[u]


def _kernel(x_h, wr_h, kT, vT, wq_h, wo_h, wg_h, wu_h, wd_h, o_ref,
            kbuf, vbuf, wq, wo, wg, wu, wd, x_v, wr_v, xs_ref, ys_ref, pbuf, xcol, qbd, hbuf,
            wsem, ksem, vsem):

    k32, v32, wq32, wo32, wg32, wu32, wd32 = (
        r.bitcast(u32) for r in (kbuf, vbuf, wq, wo, wg, wu, wd))

    def ld(ref32, *idx):
        return pltpu.bitcast(ref32[idx], bf16)

    def col(j):
        return pl.ds(pl.multiple_of(S - W + LANES * j, LANES), LANES)

    def loop(n, fn):
        lax.fori_loop(0, n, lambda i, c: (fn(i), c)[1], 0)

    def start_k(b):
        loop(NJ, lambda j: pltpu.make_async_copy(kT.at[b, :, col(j)], kbuf.at[b, j], ksem.at[b]).start())

    def wait_k(b):
        dst = kbuf.at[b]
        pltpu.make_async_copy(dst, dst, ksem.at[b]).wait()

    def piece_rows(p):
        return pl.ds(PIECE_T0[p] * LANES, (PIECE_T0[p + 1] - PIECE_T0[p]) * LANES)

    def start_v_whole(b):
        loop(NJ, lambda j: pltpu.make_async_copy(vT.at[b, :, col(j)], vbuf.at[b, j], vsem.at[b, 0]).start())

    def wait_v_whole(b):
        dst = vbuf.at[b]
        pltpu.make_async_copy(dst, dst, vsem.at[b, 0]).wait()

    def start_v_piece(b, p):
        rows = piece_rows(p)
        loop(NJ, lambda j: pltpu.make_async_copy(
            vT.at[b, rows, col(j)], vbuf.at[b, j, rows], vsem.at[b, p]).start())

    def wait_v_piece(b, p):
        dst = vbuf.at[b, :, piece_rows(p)]
        pltpu.make_async_copy(dst, dst, vsem.at[b, p]).wait()

    def start_w(src, dst, n, sem):
        loop(n, lambda c: pltpu.make_async_copy(
            src.at[:, pl.ds(pl.multiple_of(LANES * c, LANES), LANES)], dst.at[c], sem).start())

    def start_tall(src, dst, nblk, sem):
        rows = src.shape[0] // nblk

        def fn(i):
            r = pl.ds(pl.multiple_of((i // ND) * rows, 16), rows)
            c = i % ND
            pltpu.make_async_copy(src.at[r, pl.ds(pl.multiple_of(LANES * c, LANES), LANES)],
                                  dst.at[c, r], sem).start()
        loop(nblk * ND, fn)

    def wait_w(dst, sem):
        pltpu.make_async_copy(dst, dst, sem).wait()

    x_cp = pltpu.make_async_copy(x_h, x_v, wsem.at[5])
    wr_cp = pltpu.make_async_copy(wr_h, wr_v, wsem.at[6])

    start_w(wq_h, wq, NC, wsem.at[0])
    x_cp.start()
    wr_cp.start()
    start_k(0)
    x_cp.wait()
    wr_cp.wait()

    xs_ref[...] = x_v[...].astype(f32)
    wr = wr_v[...].astype(f32).reshape(1, D)
    wr_t = [jnp.broadcast_to(wr[:, LANES * n:LANES * (n + 1)], (G, LANES)) for n in range(ND)]

    row = lax.broadcasted_iota(jnp.int32, (G, LANES), 0)
    lane = lax.broadcasted_iota(jnp.int32, (G, LANES), 1)

    def head_mask(c):
        colm = lane + c * LANES
        lo = row * DH
        return (colm >= lo) & (colm < lo + DH)

    wait_w(wq, wsem.at[0])
    start_v_whole(0)
    start_tall(wo_h, wo, WO_BLOCKS, wsem.at[1])
    start_w(wg_h, wg, NF, wsem.at[2])
    start_w(wu_h, wu, NF, wsem.at[3])
    start_tall(wd_h, wd, WD_BLOCKS, wsem.at[4])

    sub8 = lax.broadcasted_iota(jnp.int32, (8, LANES), 0)
    lane8 = lax.broadcasted_iota(jnp.int32, (8, LANES), 1)

    def to_columns(x_tiles):
        for n, t in enumerate(x_tiles):
            t = t[:8].astype(f32)
            for r in range(LANES // 8):
                xcol[n * (LANES // 8) + r] = jnp.broadcast_to(
                    jnp.sum(jnp.where(lane8 - sub8 == 8 * r, t, 0.0), axis=1, keepdims=True), (8, LANES))

    def vpu_matvec(cols):
        accs = [None] * len(cols)
        for kg in range(D // 16):
            x0, x1 = xcol[2 * kg], xcol[2 * kg + 1]
            for i, (w32, c) in enumerate(cols):
                w = ld(w32, c, pl.ds(kg * 8, 8), slice(None)).astype(f32)
                accs[i] = _acc(accs[i], w[:8] * x0 + w[8:] * x1)
        return [jnp.sum(a, axis=0, keepdims=True) for a in accs]

    def ffn(x1):
        xn = _layernorm(x1)
        xnb_t = [t.astype(bf16) for t in xn]
        xnb = jnp.concatenate(xnb_t, axis=1)
        rr = functools.reduce(jnp.add, [a.astype(f32) * w for a, w in zip(xnb_t, wr_t)])
        gate = jax.nn.sigmoid(jnp.sum(rr, axis=1, keepdims=True))
        if FV:
            to_columns(xnb_t)
        for f in range(NF):
            if f in FV:
                gt, ut = (jnp.broadcast_to(t, (G, LANES)) for t in vpu_matvec([(wg32, f), (wu32, f)]))
            else:
                gt = _nn(xnb, ld(wg32, f))
                ut = _nn(xnb, ld(wu32, f))
            hbuf[f] = (gt * jax.nn.sigmoid(gt) * ut).astype(bf16)
        y = [None] * ND
        for f in range(NF):
            h = hbuf[f]
            for n in range(ND):
                y[n] = _acc(y[n], _nn(h, ld(wd32, n, _tile(f), slice(None))))
        return [a + bb + c * gate for a, bb, c in zip(x1, xn, y)]

    diag = lane8 - 2 * sub8

    def tiles(gi):
        h0, nh = GROUPS[gi]
        return range(h0 * DH // LANES, (h0 + nh) * DH // LANES)

    def attention(b, xs, first):
        xlo, xhi = (b + B - 1) % B, (b + B - 2) % B
        xn = [t.astype(bf16) for t in _layernorm(xs)]
        xnb = jnp.concatenate(xn, axis=1)
        qv = {}
        if QV:
            to_columns(xn)
            for i in range(0, len(QV), QV_BATCH):
                part = QV[i:i + QV_BATCH]
                qv.update(zip(part, vpu_matvec([(wq32, cc) for cc in part])))
        for gi in range(len(GROUPS)):
            for c, cc in enumerate(tiles(gi)):
                qt = jnp.broadcast_to(qv[cc], (G, LANES)) if cc in qv else _nn(xnb, ld(wq32, cc))
                qbd[cc] = jnp.where(head_mask(c), qt, 0.0).astype(bf16)
        if first:
            l1_dma_start(b)

        st = {}
        mxu, vpu = [], []

        def qk_step(gi, cc, j, last):
            def fn():
                t = _nn(qbd[cc], ld(k32, b, j, _tile(cc), slice(None)))[:8]
                t = _acc(st.pop(('sc', gi, j), None), t)
                if last:
                    pbuf[gi, j] = t
                else:
                    st['sc', gi, j] = t
            return fn

        def sm_step(gi):
            def fn():
                sc = [pbuf[gi, j] for j in range(NJ)]
                m = jnp.max(functools.reduce(jnp.maximum, sc), axis=1, keepdims=True)
                es = [jnp.exp((t - m) * SCALE) for t in sc]
                l = jnp.sum(functools.reduce(jnp.add, es), axis=1, keepdims=True)
                inv = 1.0 / l
                for j in range(NJ):
                    pbuf[gi, j] = es[j] * inv
            return fn

        def pv_step(gi, r, rg):
            def fn():
                if rg == 0:
                    st['pb'] = [jnp.broadcast_to(pbuf[gi, j, r:r + 1, :], (8, LANES)) for j in range(NJ)]
                g16 = (GROUPS[gi][0] + r) * (DH // 16) + rg
                cc, k = divmod(g16, LANES // 16)
                rows = pl.ds(g16 * 8, 8)
                lo = hi = None
                for j in range(NJ):
                    if first or j >= NX:
                        a, c_ = _unpack(v32[b, j, rows, :])
                        if j < NX:
                            k32[xlo, j, rows, :] = pltpu.bitcast(a, u32)
                            k32[xhi, j, rows, :] = pltpu.bitcast(c_, u32)
                    else:
                        a = pltpu.bitcast(k32[xlo, j, rows, :], f32)
                        c_ = pltpu.bitcast(k32[xhi, j, rows, :], f32)
                    lo = _acc(lo, a * st['pb'][j])
                    hi = _acc(hi, c_ * st['pb'][j])
                lo = jnp.sum(lo, axis=1, keepdims=True)
                hi = jnp.sum(hi, axis=1, keepdims=True)
                if vpu_wo(cc):
                    for n in range(ND):
                        a, c_ = _unpack(wo32[n, rows, :])
                        st['vacc', n] = _acc(st.get(('vacc', n)), a * lo + c_ * hi)
                else:
                    t = st.get(('ot', cc), jnp.zeros((8, LANES), f32))
                    t = jnp.where(diag == 16 * k, lo, t)
                    st['ot', cc] = jnp.where(diag == 16 * k + 1, hi, t)
            return fn

        def vpu_wo(cc):
            return (not first) and WV[0] > 0 and cc % WV[1] < WV[0]

        def wo_step(cc, n):
            def fn():
                if n == 0:
                    st['ot', cc] = st['ot', cc].astype(bf16)
                st['acc', n] = _acc(st.get(('acc', n)),
                                    _nn(st['ot', cc], ld(wo32, n, _tile(cc), slice(None))))
            return fn

        def wait_step(p):
            def fn():
                @pl.when(b == B - 1)
                def _():
                    wait_v_piece(b, p)

                if p == 0:
                    @pl.when(b < B - 1)
                    def _():
                        wait_v_whole(b)

                    @pl.when(b == 0)
                    def _():
                        wait_w(wo, wsem.at[1])
            return fn

        ng = len(GROUPS)
        pv_cost = PV_COST[0 if first else 1]
        if first:
            vpu += [(SM_COST, ('qk', gi), None, sm_step(gi)) for gi in range(ng)]
        else:
            vpu.append((SM_COST, ('qk', 0), None, sm_step(0)))
        for gi, (h0, nh) in enumerate(GROUPS):
            for r in range(nh):
                if not first and r == int(nh * SM_POS) and gi + 1 < ng:
                    vpu.append((SM_COST, ('qk', gi + 1), None, sm_step(gi + 1)))
                for rg in range(DH // 16):
                    g16 = (h0 + r) * (DH // 16) + rg
                    cc, k = divmod(g16, LANES // 16)
                    if first and k == 0 and cc in PIECE_T0[:-1]:
                        vpu.append((0.0, None, None, wait_step(PIECE_T0.index(cc))))
                    vpu.append((pv_cost + (8.0 if vpu_wo(cc) else 0.0), None, ('ot', cc), pv_step(gi, r, rg)))
        ahead = ng if first else K_AHEAD
        for gi in range(ng + ahead):
            if gi < ng:
                for cc in tiles(gi):
                    for j in range(NJ):
                        mxu.append((8, None, ('qk', gi), qk_step(gi, cc, j, cc == tiles(gi)[-1])))
            if gi >= ahead:
                for cc in tiles(gi - ahead):
                    for n in range(ND if not vpu_wo(cc) else 0):
                        mxu.append((8, ('ot', cc), None, wo_step(cc, n)))
        _emit(mxu, vpu)
        accs = [_acc(st.get(('vacc', n)), st['acc', n]) for n in range(ND)]
        return [x + jnp.sum(a, axis=0, keepdims=True) for x, a in zip(xs, accs)]

    def l1_dma_start(b):
        wait_k(b)

        @pl.when(b + 1 < B)
        def _():
            start_k(b + 1)

        @pl.when(b + 2 < B)
        def _():
            start_v_whole(b + 1)

        @pl.when(b + 2 == B)
        def _():
            for p in range(len(V_PIECES)):
                start_v_piece(b + 1, p)

    def l1_wait_all(b):
        @pl.when(b < B - 1)
        def _():
            wait_v_whole(b)

        for p in range(len(V_PIECES)):
            @pl.when(b == B - 1)
            def _():
                wait_v_piece(b, p)

        @pl.when(b == 0)
        def _():
            wait_w(wo, wsem.at[1])
            wait_w(wg, wsem.at[2])
            wait_w(wu, wsem.at[3])
            wait_w(wd, wsem.at[4])

    def layer(b, xs, first):
        x1 = attention(b, xs, first)
        if first:
            @pl.when(b == 0)
            def _():
                wait_w(wg, wsem.at[2])
                wait_w(wu, wsem.at[3])
                wait_w(wd, wsem.at[4])
        return ffn(x1)

    def batch(b, carry):
        x = jnp.broadcast_to(xs_ref[pl.ds(b, 1), :], (G, D))
        xs = [x[:, LANES * n:LANES * (n + 1)] for n in range(ND)]
        xs = layer(b, xs, True)
        xs = layer(b, xs, False)
        ys_ref[pl.ds(b, 1), :] = jnp.concatenate(xs, axis=1)[0:1, :]
        return carry

    lax.fori_loop(0, B, batch, 0)
    o_ref[...] = ys_ref[...].astype(o_ref.dtype)


@jax.jit
def pallas_interleave_layers__sliding_block_cached__moe_arch_mod__decode_kernel(
    A_x: jax.Array,
    A_k_cache: jax.Array,
    A_v_cache: jax.Array,
    A_wq: jax.Array,
    A_wo: jax.Array,
    B_x: jax.Array,
    B_w_r: jax.Array,
    B_w_gate: jax.Array,
    B_w_up: jax.Array,
    B_w_down: jax.Array,
):
    del B_x
    kT = jnp.swapaxes(A_k_cache, 2, 3).reshape(B, HD, S)
    vT = jnp.swapaxes(A_v_cache, 2, 3).reshape(B, HD, S)
    x = A_x.reshape(B, D)
    any_spec = pl.BlockSpec(memory_space=pl.ANY)
    out = pl.pallas_call(
        _kernel,
        in_specs=[any_spec] * 9,
        out_specs=pl.BlockSpec(memory_space=pltpu.VMEM),
        out_shape=jax.ShapeDtypeStruct((B, D), A_x.dtype),
        scratch_shapes=[
            pltpu.VMEM((B, NJ, HD, LANES), bf16),
            pltpu.VMEM((B, NJ, HD, LANES), bf16),
            pltpu.VMEM((NC, D, LANES), bf16),
            pltpu.VMEM((ND, HD, LANES), bf16),
            pltpu.VMEM((NF, D, LANES), bf16),
            pltpu.VMEM((NF, D, LANES), bf16),
            pltpu.VMEM((ND, F, LANES), bf16),
            pltpu.VMEM((B, D), bf16),
            pltpu.VMEM((D,), bf16),
            pltpu.VMEM((B, D), f32),
            pltpu.VMEM((B, D), f32),
            pltpu.VMEM((len(GROUPS), NJ, 8, LANES), f32),
            pltpu.VMEM((D // 8, 8, LANES), f32),
            pltpu.VMEM((NC, G, LANES), bf16),
            pltpu.VMEM((NF, G, LANES), bf16),
            pltpu.SemaphoreType.DMA((7,)),
            pltpu.SemaphoreType.DMA((B,)),
            pltpu.SemaphoreType.DMA((B, len(V_PIECES))),
        ],
        compiler_params=pltpu.CompilerParams(vmem_limit_bytes=126 * 1024 * 1024, flags=FLAGS),
    )(x, B_w_r, kT, vT, A_wq, A_wo, B_w_gate, B_w_up, B_w_down)
    return out.reshape(A_x.shape)
```

```python
import functools

import jax
import jax.numpy as jnp
from jax import lax
from jax.experimental import pallas as pl
from jax.experimental.pallas import tpu as pltpu

B, D, H, DH, S, F = 4, 640, 32, 192, 4096, 1536
W = min(4096, max(256, S // 4))
HD = H * DH
LANES = 128
NJ = W // LANES
NC = HD // LANES
ND = D // LANES
NF = F // LANES
EPS = 1e-5
SCALE = DH ** -0.5

G = 16
NG = H // G
CPG = G * DH // LANES
V_PIECES = (24, 12, 6, 3, 2, 1)
assert sum(V_PIECES) == NC and B % 2 == 0
PIECE_T0 = [sum(V_PIECES[:p]) for p in range(len(V_PIECES) + 1)]

GROUPS = ((0, 2), (2, 6), (8, 8), (16, 8), (24, 8))
assert sum(n for _, n in GROUPS) == H
SM_COST, DEP_LAT, K_AHEAD, SM_POS = 90.0, 90.0, 2, 0.5
PV_COST = (16.0, 8.5)
NX = 8
WV = (1, 7)
QV = tuple(range(2, NC, 3))
QV_BATCH = 2
MERGE_Q = False
FV = (3, 7, 11)

FLAGS = None
DBG = ()
WO_BLOCKS = 8
WD_BLOCKS = 2
KORDER = 'j'

bf16 = jnp.bfloat16
u32 = jnp.uint32
f32 = jnp.float32


def _nn(a, b):
    return jnp.dot(a, b, preferred_element_type=f32)


def _nt(a, b):
    return lax.dot_general(a, b, (((1,), (1,)), ((), ())), preferred_element_type=f32)


def _acc(a, t):
    return t if a is None else a + t


def _layernorm(xs):
    s1 = jnp.sum(functools.reduce(jnp.add, xs), axis=1, keepdims=True)
    s2 = jnp.sum(functools.reduce(jnp.add, [x * x for x in xs]), axis=1, keepdims=True)
    mean = s1 * (1.0 / D)
    var = jnp.maximum(s2 * (1.0 / D) - mean * mean, 0.0)
    inv = lax.rsqrt(var + EPS)
    return [(x - mean) * inv for x in xs]


def _tile(c):
    return pl.ds(c * (LANES // 2), LANES // 2)


def _unpack(w):
    lo = pltpu.bitcast(w << 16, f32)
    hi = pltpu.bitcast(w & jnp.uint32(0xFFFF0000), f32)
    return lo, hi


def _emit(mxu, vpu):
    remaining, done = {}, {}
    for s in mxu + vpu:
        if s[2] is not None:
            remaining[s[2]] = remaining.get(s[2], 0) + 1
    t = [0.0, 0.0]
    idx = [0, 0]
    streams = (mxu, vpu)
    while idx[0] < len(mxu) or idx[1] < len(vpu):
        start = []
        for u in (0, 1):
            if idx[u] >= len(streams[u]):
                start.append(None)
                continue
            dep = streams[u][idx[u]][1]
            if dep is None or dep not in remaining:
                start.append(t[u])
            elif dep in done:
                start.append(max(t[u], done[dep] + DEP_LAT))
            else:
                start.append(None)
        u = min((u for u in (0, 1) if start[u] is not None), key=lambda u: start[u])
        cost, _, tag, fn = streams[u][idx[u]]
        idx[u] += 1
        fn()
        t[u] = start[u] + cost
        if tag is not None:
            remaining[tag] -= 1
            if remaining[tag] == 0:
                done[tag] = t[u]


def _kernel(x_h, wr_h, kT, vT, wq_h, wo_h, wg_h, wu_h, wd_h, o_ref,
            kbuf, vbuf, wq, wo, wg, wu, wd, x_v, wr_v, xs_ref, ys_ref, pbuf, xcol, qbd, hbuf,
            sems):

    k32, v32, wq32, wo32, wg32, wu32, wd32 = (
        r.bitcast(u32) for r in (kbuf, vbuf, wq, wo, wg, wu, wd))

    ksem = sems.at[0]
    wsem_q, wsem_x, wsem_o, wsem_f = sems.at[3], sems.at[4], sems.at[5], sems.at[6]

    def vsem_whole(b):
        return sems.at[1 + b % 2]

    def vsem_piece(p):
        return sems.at[2 + p]

    def ld(ref32, *idx):
        return pltpu.bitcast(ref32[idx], bf16)

    def col(j):
        return pl.ds(pl.multiple_of(S - W + LANES * j, LANES), LANES)

    def loop(n, fn):
        lax.fori_loop(0, n, lambda i, c: (fn(i), c)[1], 0)

    def start_k(b):
        loop(NJ, lambda j: pltpu.make_async_copy(kT.at[b, :, col(j)], kbuf.at[b, j], ksem).start())

    def wait_k(b):
        dst = kbuf.at[b]
        pltpu.make_async_copy(dst, dst, ksem).wait()

    def piece_rows(p):
        return pl.ds(PIECE_T0[p] * LANES, (PIECE_T0[p + 1] - PIECE_T0[p]) * LANES)

    def start_v_whole(b):
        loop(NJ, lambda j: pltpu.make_async_copy(vT.at[b, :, col(j)], vbuf.at[b, j], vsem_whole(b)).start())

    def wait_v_whole(b):
        dst = vbuf.at[b]
        pltpu.make_async_copy(dst, dst, vsem_whole(b)).wait()

    def start_v_piece(b, p):
        rows = piece_rows(p)
        loop(NJ, lambda j: pltpu.make_async_copy(
            vT.at[b, rows, col(j)], vbuf.at[b, j, rows], vsem_piece(p)).start())

    def wait_v_piece(b, p):
        dst = vbuf.at[b, :, piece_rows(p)]
        pltpu.make_async_copy(dst, dst, vsem_piece(p)).wait()

    def start_w(src, dst, n, sem):
        loop(n, lambda c: pltpu.make_async_copy(
            src.at[:, pl.ds(pl.multiple_of(LANES * c, LANES), LANES)], dst.at[c], sem).start())

    def start_tall(src, dst, nblk, sem):
        rows = src.shape[0] // nblk

        def fn(i):
            r = pl.ds(pl.multiple_of((i // ND) * rows, 16), rows)
            c = i % ND
            pltpu.make_async_copy(src.at[r, pl.ds(pl.multiple_of(LANES * c, LANES), LANES)],
                                  dst.at[c, r], sem).start()
        loop(nblk * ND, fn)

    def wait_w(dst, sem):
        pltpu.make_async_copy(dst, dst, sem).wait()

    x_cp = pltpu.make_async_copy(x_h, x_v, wsem_x)
    wr_cp = pltpu.make_async_copy(wr_h, wr_v, wsem_x)

    start_w(wq_h, wq, NC, wsem_q)
    x_cp.start()
    wr_cp.start()
    start_k(0)
    x_cp.wait()
    wr_cp.wait()

    xs_ref[...] = x_v[...].astype(f32)
    wr = wr_v[...].astype(f32).reshape(1, D)
    wr_t = [jnp.broadcast_to(wr[:, LANES * n:LANES * (n + 1)], (G, LANES)) for n in range(ND)]

    row = lax.broadcasted_iota(jnp.int32, (G, LANES), 0)
    lane = lax.broadcasted_iota(jnp.int32, (G, LANES), 1)

    def head_mask(c):
        colm = lane + c * LANES
        lo = row * DH
        return (colm >= lo) & (colm < lo + DH)

    wait_w(wq, wsem_q)
    start_v_whole(0)
    start_tall(wo_h, wo, WO_BLOCKS, wsem_o)
    start_w(wg_h, wg, NF, wsem_f)
    start_w(wu_h, wu, NF, wsem_f)
    start_tall(wd_h, wd, WD_BLOCKS, wsem_f)

    sub8 = lax.broadcasted_iota(jnp.int32, (8, LANES), 0)
    lane8 = lax.broadcasted_iota(jnp.int32, (8, LANES), 1)

    def to_columns(x_tiles):
        for n, t in enumerate(x_tiles):
            t = t[:8].astype(f32)
            for r in range(LANES // 8):
                xcol[n * (LANES // 8) + r] = jnp.broadcast_to(
                    jnp.sum(jnp.where(lane8 - sub8 == 8 * r, t, 0.0), axis=1, keepdims=True), (8, LANES))

    def vpu_matvec(cols):
        accs = [None] * len(cols)
        for kg in range(D // 16):
            x0, x1 = xcol[2 * kg], xcol[2 * kg + 1]
            for i, (w32, c) in enumerate(cols):
                w = ld(w32, c, pl.ds(kg * 8, 8), slice(None)).astype(f32)
                accs[i] = _acc(accs[i], w[:8] * x0 + w[8:] * x1)
        return [jnp.sum(a, axis=0, keepdims=True) for a in accs]

    def ffn(x1):
        xn = _layernorm(x1)
        xnb_t = [t.astype(bf16) for t in xn]
        xnb = jnp.concatenate(xnb_t, axis=1)
        rr = functools.reduce(jnp.add, [a.astype(f32) * w for a, w in zip(xnb_t, wr_t)])
        gate = jax.nn.sigmoid(jnp.sum(rr, axis=1, keepdims=True))
        if FV:
            to_columns(xnb_t)
        for f in range(NF):
            if f in FV:
                gt, ut = (jnp.broadcast_to(t, (G, LANES)) for t in vpu_matvec([(wg32, f), (wu32, f)]))
            else:
                gt = _nn(xnb, ld(wg32, f))
                ut = _nn(xnb, ld(wu32, f))
            hbuf[f] = (gt * jax.nn.sigmoid(gt) * ut).astype(bf16)
        y = [None] * ND
        for f in range(NF):
            h = hbuf[f]
            for n in range(ND):
                y[n] = _acc(y[n], _nn(h, ld(wd32, n, _tile(f), slice(None))))
        return [a + bb + c * gate for a, bb, c in zip(x1, xn, y)]

    diag = lane8 - 2 * sub8

    def tiles(gi):
        h0, nh = GROUPS[gi]
        return range(h0 * DH // LANES, (h0 + nh) * DH // LANES)

    def attention(b, xs, first):
        xlo, xhi = (b + B - 1) % B, (b + B - 2) % B
        xn = [t.astype(bf16) for t in _layernorm(xs)]
        xnb = jnp.concatenate(xn, axis=1)
        qv = {}

        def q_step(gi, c, cc):
            def fn():
                qt = jnp.broadcast_to(qv[cc], (G, LANES)) if cc in qv else _nn(xnb, ld(wq32, cc))
                qbd[cc] = jnp.where(head_mask(c), qt, 0.0).astype(bf16)
            return fn

        merge_q = MERGE_Q and not first
        if not merge_q:
            if QV:
                to_columns(xn)
                for i in range(0, len(QV), QV_BATCH):
                    part = QV[i:i + QV_BATCH]
                    qv.update(zip(part, vpu_matvec([(wq32, cc) for cc in part])))
            for gi in range(len(GROUPS)):
                for c, cc in enumerate(tiles(gi)):
                    q_step(gi, c, cc)()
        if first:
            l1_dma_start(b)

        st = {}
        mxu, vpu = [], []

        def qk_step(gi, cc, j, last):
            def fn():
                t = _nn(qbd[cc], ld(k32, b, j, _tile(cc), slice(None)))[:8]
                t = _acc(st.pop(('sc', gi, j), None), t)
                if last:
                    pbuf[gi, j] = t
                else:
                    st['sc', gi, j] = t
            return fn

        def sm_step(gi):
            def fn():
                sc = [pbuf[gi, j] for j in range(NJ)]
                m = jnp.max(functools.reduce(jnp.maximum, sc), axis=1, keepdims=True)
                es = [jnp.exp((t - m) * SCALE) for t in sc]
                l = jnp.sum(functools.reduce(jnp.add, es), axis=1, keepdims=True)
                inv = 1.0 / l
                for j in range(NJ):
                    pbuf[gi, j] = es[j] * inv
            return fn

        def pv_step(gi, r, rg):
            def fn():
                if rg == 0:
                    st['pb'] = [jnp.broadcast_to(pbuf[gi, j, r:r + 1, :], (8, LANES)) for j in range(NJ)]
                g16 = (GROUPS[gi][0] + r) * (DH // 16) + rg
                cc, k = divmod(g16, LANES // 16)
                rows = pl.ds(g16 * 8, 8)
                lo = hi = None
                for j in range(NJ):
                    if first or j >= NX:
                        a, c_ = _unpack(v32[b, j, rows, :])
                        if j < NX:
                            k32[xlo, j, rows, :] = pltpu.bitcast(a, u32)
                            k32[xhi, j, rows, :] = pltpu.bitcast(c_, u32)
                    else:
                        a = pltpu.bitcast(k32[xlo, j, rows, :], f32)
                        c_ = pltpu.bitcast(k32[xhi, j, rows, :], f32)
                    lo = _acc(lo, a * st['pb'][j])
                    hi = _acc(hi, c_ * st['pb'][j])
                lo = jnp.sum(lo, axis=1, keepdims=True)
                hi = jnp.sum(hi, axis=1, keepdims=True)
                if vpu_wo(cc):
                    for n in range(ND):
                        a, c_ = _unpack(wo32[n, rows, :])
                        st['vacc', n] = _acc(st.get(('vacc', n)), a * lo + c_ * hi)
                else:
                    t = st.get(('ot', cc), jnp.zeros((8, LANES), f32))
                    t = jnp.where(diag == 16 * k, lo, t)
                    st['ot', cc] = jnp.where(diag == 16 * k + 1, hi, t)
            return fn

        def vpu_wo(cc):
            return (not first) and WV[0] > 0 and cc % WV[1] < WV[0]

        def wo_step(cc, n):
            def fn():
                if n == 0:
                    st['ot', cc] = st['ot', cc].astype(bf16)
                st['acc', n] = _acc(st.get(('acc', n)),
                                    _nn(st['ot', cc], ld(wo32, n, _tile(cc), slice(None))))
            return fn

        def wait_step(p):
            def fn():
                @pl.when(b == B - 1)
                def _():
                    wait_v_piece(b, p)

                if p == 0:
                    @pl.when(b < B - 1)
                    def _():
                        wait_v_whole(b)

                    @pl.when(b == 0)
                    def _():
                        wait_w(wo, wsem_o)
            return fn

        ng = len(GROUPS)
        pv_cost = PV_COST[0 if first else 1]
        if first:
            vpu += [(SM_COST, ('qk', gi), None, sm_step(gi)) for gi in range(ng)]
        else:
            vpu.append((SM_COST, ('qk', 0), None, sm_step(0)))
        for gi, (h0, nh) in enumerate(GROUPS):
            for r in range(nh):
                if not first and r == int(nh * SM_POS) and gi + 1 < ng:
                    vpu.append((SM_COST, ('qk', gi + 1), None, sm_step(gi + 1)))
                for rg in range(DH // 16):
                    g16 = (h0 + r) * (DH // 16) + rg
                    cc, k = divmod(g16, LANES // 16)
                    if first and k == 0 and cc in PIECE_T0[:-1]:
                        vpu.append((0.0, None, None, wait_step(PIECE_T0.index(cc))))
                    vpu.append((pv_cost + (8.0 if vpu_wo(cc) else 0.0), None, ('ot', cc), pv_step(gi, r, rg)))
        ahead = ng if first else K_AHEAD
        def add_q(gi):
            if merge_q and gi < ng:
                for c, cc in enumerate(tiles(gi)):
                    mxu.append((40, None, None, q_step(gi, c, cc)))

        add_q(0)
        for gi in range(ng + ahead):
            add_q(gi + 1)
            if gi < ng:
                for cc in tiles(gi):
                    for j in range(NJ):
                        mxu.append((8, None, ('qk', gi), qk_step(gi, cc, j, cc == tiles(gi)[-1])))
            if gi >= ahead:
                for cc in tiles(gi - ahead):
                    for n in range(ND if not vpu_wo(cc) else 0):
                        mxu.append((8, ('ot', cc), None, wo_step(cc, n)))
        _emit(mxu, vpu)
        accs = [_acc(st.get(('vacc', n)), st['acc', n]) for n in range(ND)]
        return [x + jnp.sum(a, axis=0, keepdims=True) for x, a in zip(xs, accs)]

    def l1_dma_start(b):
        wait_k(b)

        @pl.when(b + 1 < B)
        def _():
            start_k(b + 1)

        @pl.when(b + 2 < B)
        def _():
            start_v_whole(b + 1)

        @pl.when(b + 2 == B)
        def _():
            for p in range(len(V_PIECES)):
                start_v_piece(b + 1, p)

    def l1_wait_all(b):
        @pl.when(b < B - 1)
        def _():
            wait_v_whole(b)

        for p in range(len(V_PIECES)):
            @pl.when(b == B - 1)
            def _():
                wait_v_piece(b, p)

        @pl.when(b == 0)
        def _():
            wait_w(wo, wsem_o)
            wait_w(wg, wsem_f)
            wait_w(wu, wsem_f)
            wait_w(wd, wsem_f)

    def layer(b, xs, first):
        x1 = attention(b, xs, first)
        if first:
            @pl.when(b == 0)
            def _():
                wait_w(wg, wsem_f)
                wait_w(wu, wsem_f)
                wait_w(wd, wsem_f)
        return ffn(x1)

    def batch(b, carry):
        x = jnp.broadcast_to(xs_ref[pl.ds(b, 1), :], (G, D))
        xs = [x[:, LANES * n:LANES * (n + 1)] for n in range(ND)]
        xs = layer(b, xs, True)
        xs = layer(b, xs, False)
        ys_ref[pl.ds(b, 1), :] = jnp.concatenate(xs, axis=1)[0:1, :]
        return carry

    lax.fori_loop(0, B, batch, 0)
    o_ref[...] = ys_ref[...].astype(o_ref.dtype)


@jax.jit
def pallas_interleave_layers__sliding_block_cached__moe_arch_mod__decode_kernel(
    A_x: jax.Array,
    A_k_cache: jax.Array,
    A_v_cache: jax.Array,
    A_wq: jax.Array,
    A_wo: jax.Array,
    B_x: jax.Array,
    B_w_r: jax.Array,
    B_w_gate: jax.Array,
    B_w_up: jax.Array,
    B_w_down: jax.Array,
):
    del B_x
    kT = jnp.swapaxes(A_k_cache, 2, 3).reshape(B, HD, S)
    vT = jnp.swapaxes(A_v_cache, 2, 3).reshape(B, HD, S)
    x = A_x.reshape(B, D)
    any_spec = pl.BlockSpec(memory_space=pl.ANY)
    out = pl.pallas_call(
        _kernel,
        in_specs=[any_spec] * 9,
        out_specs=pl.BlockSpec(memory_space=pltpu.VMEM),
        out_shape=jax.ShapeDtypeStruct((B, D), A_x.dtype),
        scratch_shapes=[
            pltpu.VMEM((B, NJ, HD, LANES), bf16),
            pltpu.VMEM((B, NJ, HD, LANES), bf16),
            pltpu.VMEM((NC, D, LANES), bf16),
            pltpu.VMEM((ND, HD, LANES), bf16),
            pltpu.VMEM((NF, D, LANES), bf16),
            pltpu.VMEM((NF, D, LANES), bf16),
            pltpu.VMEM((ND, F, LANES), bf16),
            pltpu.VMEM((B, D), bf16),
            pltpu.VMEM((D,), bf16),
            pltpu.VMEM((B, D), f32),
            pltpu.VMEM((B, D), f32),
            pltpu.VMEM((len(GROUPS), NJ, 8, LANES), f32),
            pltpu.VMEM((D // 8, 8, LANES), f32),
            pltpu.VMEM((NC, G, LANES), bf16),
            pltpu.VMEM((NF, G, LANES), bf16),
            pltpu.SemaphoreType.DMA((max(7, 2 + len(V_PIECES)),)),
        ],
        compiler_params=pltpu.CompilerParams(vmem_limit_bytes=126 * 1024 * 1024, flags=FLAGS),
    )(x, B_w_r, kT, vT, A_wq, A_wo, B_w_gate, B_w_up, B_w_down)
    return out.reshape(A_x.shape)
```

```python
import functools

import jax
import jax.numpy as jnp
from jax import lax
from jax.experimental import pallas as pl
from jax.experimental.pallas import tpu as pltpu

B, D, H, DH, S, F = 4, 640, 32, 192, 4096, 1536
W = min(4096, max(256, S // 4))
HD = H * DH
LANES = 128
NJ = W // LANES
NC = HD // LANES
ND = D // LANES
NF = F // LANES
EPS = 1e-5
SCALE = DH ** -0.5

G = 16
V_PIECES = (24, 12, 6, 3, 2, 1)
assert sum(V_PIECES) == NC and B % 2 == 0
PIECE_T0 = [sum(V_PIECES[:p]) for p in range(len(V_PIECES) + 1)]

GROUPS = ((0, 4), (4, 4), (8, 4), (12, 4), (16, 4), (20, 6), (26, 6))
assert sum(n for _, n in GROUPS) == H
SM_COST, DEP_LAT, K_AHEAD, SM_POS = 90.0, 90.0, 2, 0.5
PV_COST = (16.0, 8.5)
WV_PERIOD = 7
QV = tuple(range(2, NC, 3))
QV_BATCH = 2
FV = (5, 11)
WO_BLOCKS = 8
WD_BLOCKS = 2

bf16 = jnp.bfloat16
u32 = jnp.uint32
f32 = jnp.float32


def _nn(a, b):
    return jnp.dot(a, b, preferred_element_type=f32)


def _acc(a, t):
    return t if a is None else a + t


def _layernorm(xs):
    s1 = jnp.sum(functools.reduce(jnp.add, xs), axis=1, keepdims=True)
    s2 = jnp.sum(functools.reduce(jnp.add, [x * x for x in xs]), axis=1, keepdims=True)
    mean = s1 * (1.0 / D)
    var = jnp.maximum(s2 * (1.0 / D) - mean * mean, 0.0)
    inv = lax.rsqrt(var + EPS)
    return [(x - mean) * inv for x in xs]


def _tile(c):
    return pl.ds(c * (LANES // 2), LANES // 2)


def _unpack(w):
    lo = pltpu.bitcast(w << 16, f32)
    hi = pltpu.bitcast(w & jnp.uint32(0xFFFF0000), f32)
    return lo, hi


def _emit(mxu, vpu):
    remaining, done = {}, {}
    for s in mxu + vpu:
        if s[2] is not None:
            remaining[s[2]] = remaining.get(s[2], 0) + 1
    t = [0.0, 0.0]
    idx = [0, 0]
    streams = (mxu, vpu)
    while idx[0] < len(mxu) or idx[1] < len(vpu):
        start = []
        for u in (0, 1):
            if idx[u] >= len(streams[u]):
                start.append(None)
                continue
            dep = streams[u][idx[u]][1]
            if dep is None or dep not in remaining:
                start.append(t[u])
            elif dep in done:
                start.append(max(t[u], done[dep] + DEP_LAT))
            else:
                start.append(None)
        u = min((u for u in (0, 1) if start[u] is not None), key=lambda u: start[u])
        cost, _, tag, fn = streams[u][idx[u]]
        idx[u] += 1
        fn()
        t[u] = start[u] + cost
        if tag is not None:
            remaining[tag] -= 1
            if remaining[tag] == 0:
                done[tag] = t[u]


def _kernel(x_h, wr_h, kT, vT, wq_h, wo_h, wg_h, wu_h, wd_h, o_ref,
            kbuf, vbuf, wq, wo, wg, wu, wd, x_v, wr_v, xs_ref, ys_ref, pbuf, xcol, qbd, hbuf,
            sems):

    k32, v32, wq32, wo32, wg32, wu32, wd32 = (
        r.bitcast(u32) for r in (kbuf, vbuf, wq, wo, wg, wu, wd))

    ksem = sems.at[0]
    wsem_q, wsem_x, wsem_o, wsem_f = sems.at[3], sems.at[4], sems.at[5], sems.at[6]

    def vsem_whole(b):
        return sems.at[1 + b % 2]

    def vsem_piece(p):
        return sems.at[2 + p]

    def ld(ref32, *idx):
        return pltpu.bitcast(ref32[idx], bf16)

    def col(j):
        return pl.ds(pl.multiple_of(S - W + LANES * j, LANES), LANES)

    def loop(n, fn):
        lax.fori_loop(0, n, lambda i, c: (fn(i), c)[1], 0)

    def start_k(b):
        loop(NJ, lambda j: pltpu.make_async_copy(kT.at[b, :, col(j)], kbuf.at[b, j], ksem).start())

    def wait_k(b):
        dst = kbuf.at[b]
        pltpu.make_async_copy(dst, dst, ksem).wait()

    def piece_rows(p):
        return pl.ds(PIECE_T0[p] * LANES, (PIECE_T0[p + 1] - PIECE_T0[p]) * LANES)

    def start_v_whole(b):
        loop(NJ, lambda j: pltpu.make_async_copy(vT.at[b, :, col(j)], vbuf.at[b, j], vsem_whole(b)).start())

    def wait_v_whole(b):
        dst = vbuf.at[b]
        pltpu.make_async_copy(dst, dst, vsem_whole(b)).wait()

    def start_v_piece(b, p):
        rows = piece_rows(p)
        loop(NJ, lambda j: pltpu.make_async_copy(
            vT.at[b, rows, col(j)], vbuf.at[b, j, rows], vsem_piece(p)).start())

    def wait_v_piece(b, p):
        dst = vbuf.at[b, :, piece_rows(p)]
        pltpu.make_async_copy(dst, dst, vsem_piece(p)).wait()

    def start_w(src, dst, n, sem):
        loop(n, lambda c: pltpu.make_async_copy(
            src.at[:, pl.ds(pl.multiple_of(LANES * c, LANES), LANES)], dst.at[c], sem).start())

    def start_tall(src, dst, nblk, sem):
        rows = src.shape[0] // nblk

        def fn(i):
            r = pl.ds(pl.multiple_of((i // ND) * rows, 16), rows)
            c = i % ND
            pltpu.make_async_copy(src.at[r, pl.ds(pl.multiple_of(LANES * c, LANES), LANES)],
                                  dst.at[c, r], sem).start()
        loop(nblk * ND, fn)

    def wait_w(dst, sem):
        pltpu.make_async_copy(dst, dst, sem).wait()

    x_cp = pltpu.make_async_copy(x_h, x_v, wsem_x)
    wr_cp = pltpu.make_async_copy(wr_h, wr_v, wsem_x)

    start_w(wq_h, wq, NC, wsem_q)
    x_cp.start()
    wr_cp.start()
    start_k(0)
    x_cp.wait()
    wr_cp.wait()

    xs_ref[...] = x_v[...].astype(f32)
    wr = wr_v[...].astype(f32).reshape(1, D)
    wr_t = [jnp.broadcast_to(wr[:, LANES * n:LANES * (n + 1)], (G, LANES)) for n in range(ND)]

    row = lax.broadcasted_iota(jnp.int32, (G, LANES), 0)
    lane = lax.broadcasted_iota(jnp.int32, (G, LANES), 1)

    def head_mask(c):
        colm = lane + c * LANES
        lo = row * DH
        return (colm >= lo) & (colm < lo + DH)

    wait_w(wq, wsem_q)
    start_v_whole(0)
    start_tall(wo_h, wo, WO_BLOCKS, wsem_o)
    start_w(wg_h, wg, NF, wsem_f)
    start_w(wu_h, wu, NF, wsem_f)
    start_tall(wd_h, wd, WD_BLOCKS, wsem_f)

    sub8 = lax.broadcasted_iota(jnp.int32, (8, LANES), 0)
    lane8 = lax.broadcasted_iota(jnp.int32, (8, LANES), 1)

    def to_columns(x_tiles):
        for n, t in enumerate(x_tiles):
            t = t[:8].astype(f32)
            for r in range(LANES // 8):
                xcol[n * (LANES // 8) + r] = jnp.broadcast_to(
                    jnp.sum(jnp.where(lane8 - sub8 == 8 * r, t, 0.0), axis=1, keepdims=True), (8, LANES))

    def vpu_matvec(cols):
        accs = [None] * len(cols)
        for kg in range(D // 16):
            x0, x1 = xcol[2 * kg], xcol[2 * kg + 1]
            for i, (w32, c) in enumerate(cols):
                w = ld(w32, c, pl.ds(kg * 8, 8), slice(None)).astype(f32)
                accs[i] = _acc(accs[i], w[:8] * x0 + w[8:] * x1)
        return [jnp.sum(a, axis=0, keepdims=True) for a in accs]

    def ffn(x1):
        xn = _layernorm(x1)
        xnb_t = [t.astype(bf16) for t in xn]
        xnb = jnp.concatenate(xnb_t, axis=1)
        rr = functools.reduce(jnp.add, [a.astype(f32) * w for a, w in zip(xnb_t, wr_t)])
        gate = jax.nn.sigmoid(jnp.sum(rr, axis=1, keepdims=True))
        to_columns(xnb_t)
        for f in range(NF):
            if f in FV:
                gt, ut = (jnp.broadcast_to(t, (G, LANES)) for t in vpu_matvec([(wg32, f), (wu32, f)]))
            else:
                gt = _nn(xnb, ld(wg32, f))
                ut = _nn(xnb, ld(wu32, f))
            hbuf[f] = (gt * jax.nn.sigmoid(gt) * ut).astype(bf16)
        y = [None] * ND
        for f in range(NF):
            h = hbuf[f]
            for n in range(ND):
                y[n] = _acc(y[n], _nn(h, ld(wd32, n, _tile(f), slice(None))))
        return [a + bb + c * gate for a, bb, c in zip(x1, xn, y)]

    diag = lane8 - 2 * sub8

    def tiles(gi):
        h0, nh = GROUPS[gi]
        return range(h0 * DH // LANES, (h0 + nh) * DH // LANES)

    def attention(b, xs, first):
        xlo, xhi = (b + B - 1) % B, (b + B - 2) % B
        xn = [t.astype(bf16) for t in _layernorm(xs)]
        xnb = jnp.concatenate(xn, axis=1)
        qv = {}

        to_columns(xn)
        for i in range(0, len(QV), QV_BATCH):
            part = QV[i:i + QV_BATCH]
            qv.update(zip(part, vpu_matvec([(wq32, cc) for cc in part])))
        for gi in range(len(GROUPS)):
            for c, cc in enumerate(tiles(gi)):
                qt = jnp.broadcast_to(qv[cc], (G, LANES)) if cc in qv else _nn(xnb, ld(wq32, cc))
                qbd[cc] = jnp.where(head_mask(c), qt, 0.0).astype(bf16)
        if first:
            l1_dma_start(b)

        st = {}
        mxu, vpu = [], []

        def qk_step(gi, cc, j, last):
            def fn():
                t = _nn(qbd[cc], ld(k32, b, j, _tile(cc), slice(None)))[:8]
                t = _acc(st.pop(('sc', gi, j), None), t)
                if last:
                    pbuf[gi, j] = t
                else:
                    st['sc', gi, j] = t
            return fn

        def sm_step(gi):
            def fn():
                sc = [pbuf[gi, j] for j in range(NJ)]
                m = jnp.max(functools.reduce(jnp.maximum, sc), axis=1, keepdims=True)
                es = [jnp.exp((t - m) * SCALE) for t in sc]
                l = jnp.sum(functools.reduce(jnp.add, es), axis=1, keepdims=True)
                inv = 1.0 / l
                for j in range(NJ):
                    pbuf[gi, j] = es[j] * inv
            return fn

        def pv_step(gi, r, rg):
            def fn():
                if rg == 0:
                    st['pb'] = [jnp.broadcast_to(pbuf[gi, j, r:r + 1, :], (8, LANES)) for j in range(NJ)]
                g16 = (GROUPS[gi][0] + r) * (DH // 16) + rg
                cc, k = divmod(g16, LANES // 16)
                rows = pl.ds(g16 * 8, 8)
                lo = hi = None
                for j in range(NJ):
                    if first:
                        a, c_ = _unpack(v32[b, j, rows, :])
                        k32[xlo, j, rows, :] = pltpu.bitcast(a, u32)
                        k32[xhi, j, rows, :] = pltpu.bitcast(c_, u32)
                    else:
                        a = pltpu.bitcast(k32[xlo, j, rows, :], f32)
                        c_ = pltpu.bitcast(k32[xhi, j, rows, :], f32)
                    lo = _acc(lo, a * st['pb'][j])
                    hi = _acc(hi, c_ * st['pb'][j])
                lo = jnp.sum(lo, axis=1, keepdims=True)
                hi = jnp.sum(hi, axis=1, keepdims=True)
                if vpu_wo(cc):
                    for n in range(ND):
                        a, c_ = _unpack(wo32[n, rows, :])
                        st['vacc', n] = _acc(st.get(('vacc', n)), a * lo + c_ * hi)
                else:
                    t = st.get(('ot', cc), jnp.zeros((8, LANES), f32))
                    t = jnp.where(diag == 16 * k, lo, t)
                    st['ot', cc] = jnp.where(diag == 16 * k + 1, hi, t)
            return fn

        def vpu_wo(cc):
            return (not first) and cc % WV_PERIOD == 0

        def wo_step(cc, n):
            def fn():
                if n == 0:
                    st['ot', cc] = st['ot', cc].astype(bf16)
                st['acc', n] = _acc(st.get(('acc', n)),
                                    _nn(st['ot', cc], ld(wo32, n, _tile(cc), slice(None))))
            return fn

        def wait_step(p):
            def fn():
                @pl.when(b == B - 1)
                def _():
                    wait_v_piece(b, p)

                if p == 0:
                    @pl.when(b < B - 1)
                    def _():
                        wait_v_whole(b)

                    @pl.when(b == 0)
                    def _():
                        wait_w(wo, wsem_o)
            return fn

        ng = len(GROUPS)
        pv_cost = PV_COST[0 if first else 1]
        if first:
            vpu += [(SM_COST, ('qk', gi), None, sm_step(gi)) for gi in range(ng)]
        else:
            vpu.append((SM_COST, ('qk', 0), None, sm_step(0)))
        for gi, (h0, nh) in enumerate(GROUPS):
            for r in range(nh):
                if not first and r == int(nh * SM_POS) and gi + 1 < ng:
                    vpu.append((SM_COST, ('qk', gi + 1), None, sm_step(gi + 1)))
                for rg in range(DH // 16):
                    g16 = (h0 + r) * (DH // 16) + rg
                    cc, k = divmod(g16, LANES // 16)
                    if first and k == 0 and cc in PIECE_T0[:-1]:
                        vpu.append((0.0, None, None, wait_step(PIECE_T0.index(cc))))
                    vpu.append((pv_cost + (8.0 if vpu_wo(cc) else 0.0), None, ('ot', cc), pv_step(gi, r, rg)))
        ahead = ng if first else K_AHEAD
        for gi in range(ng + ahead):
            if gi < ng:
                for cc in tiles(gi):
                    for j in range(NJ):
                        mxu.append((8, None, ('qk', gi), qk_step(gi, cc, j, cc == tiles(gi)[-1])))
            if gi >= ahead:
                for cc in tiles(gi - ahead):
                    for n in range(ND if not vpu_wo(cc) else 0):
                        mxu.append((8, ('ot', cc), None, wo_step(cc, n)))
        _emit(mxu, vpu)
        accs = [_acc(st.get(('vacc', n)), st['acc', n]) for n in range(ND)]
        return [x + jnp.sum(a, axis=0, keepdims=True) for x, a in zip(xs, accs)]

    def l1_dma_start(b):
        wait_k(b)

        @pl.when(b + 1 < B)
        def _():
            start_k(b + 1)

        @pl.when(b + 2 < B)
        def _():
            start_v_whole(b + 1)

        @pl.when(b + 2 == B)
        def _():
            for p in range(len(V_PIECES)):
                start_v_piece(b + 1, p)

    def layer(b, xs, first):
        x1 = attention(b, xs, first)
        if first:
            @pl.when(b == 0)
            def _():
                wait_w(wg, wsem_f)
                wait_w(wu, wsem_f)
                wait_w(wd, wsem_f)
        return ffn(x1)

    def batch(b, carry):
        x = jnp.broadcast_to(xs_ref[pl.ds(b, 1), :], (G, D))
        xs = [x[:, LANES * n:LANES * (n + 1)] for n in range(ND)]
        xs = layer(b, xs, True)
        xs = layer(b, xs, False)
        ys_ref[pl.ds(b, 1), :] = jnp.concatenate(xs, axis=1)[0:1, :]
        return carry

    lax.fori_loop(0, B, batch, 0)
    o_ref[...] = ys_ref[...].astype(o_ref.dtype)


@jax.jit
def pallas_interleave_layers__sliding_block_cached__moe_arch_mod__decode_kernel(
    A_x: jax.Array,
    A_k_cache: jax.Array,
    A_v_cache: jax.Array,
    A_wq: jax.Array,
    A_wo: jax.Array,
    B_x: jax.Array,
    B_w_r: jax.Array,
    B_w_gate: jax.Array,
    B_w_up: jax.Array,
    B_w_down: jax.Array,
):
    del B_x
    kT = jnp.swapaxes(A_k_cache, 2, 3).reshape(B, HD, S)
    vT = jnp.swapaxes(A_v_cache, 2, 3).reshape(B, HD, S)
    x = A_x.reshape(B, D)
    any_spec = pl.BlockSpec(memory_space=pl.ANY)
    out = pl.pallas_call(
        _kernel,
        in_specs=[any_spec] * 9,
        out_specs=pl.BlockSpec(memory_space=pltpu.VMEM),
        out_shape=jax.ShapeDtypeStruct((B, D), A_x.dtype),
        scratch_shapes=[
            pltpu.VMEM((B, NJ, HD, LANES), bf16),
            pltpu.VMEM((B, NJ, HD, LANES), bf16),
            pltpu.VMEM((NC, D, LANES), bf16),
            pltpu.VMEM((ND, HD, LANES), bf16),
            pltpu.VMEM((NF, D, LANES), bf16),
            pltpu.VMEM((NF, D, LANES), bf16),
            pltpu.VMEM((ND, F, LANES), bf16),
            pltpu.VMEM((B, D), bf16),
            pltpu.VMEM((D,), bf16),
            pltpu.VMEM((B, D), f32),
            pltpu.VMEM((B, D), f32),
            pltpu.VMEM((len(GROUPS), NJ, 8, LANES), f32),
            pltpu.VMEM((D // 8, 8, LANES), f32),
            pltpu.VMEM((NC, G, LANES), bf16),
            pltpu.VMEM((NF, G, LANES), bf16),
            pltpu.SemaphoreType.DMA((max(7, 2 + len(V_PIECES)),)),
        ],
        compiler_params=pltpu.CompilerParams(vmem_limit_bytes=126 * 1024 * 1024),
    )(x, B_w_r, kT, vT, A_wq, A_wo, B_w_gate, B_w_up, B_w_down)
    return out.reshape(A_x.shape)
```

```python
import functools

import jax
import jax.numpy as jnp
from jax import lax
from jax.experimental import pallas as pl
from jax.experimental.pallas import tpu as pltpu

B, D, H, DH, S, F = 4, 640, 32, 192, 4096, 1536
W = min(4096, max(256, S // 4))
HD = H * DH
LANES = 128
NJ = W // LANES
NC = HD // LANES
ND = D // LANES
NF = F // LANES
EPS = 1e-5
SCALE = DH ** -0.5

G = 16
V_PIECES = (24, 12, 6, 3, 2, 1)
assert sum(V_PIECES) == NC and B % 2 == 0
PIECE_T0 = [sum(V_PIECES[:p]) for p in range(len(V_PIECES) + 1)]

GROUPS = ((0, 4), (4, 4), (8, 4), (12, 4), (16, 4), (20, 6), (26, 6))
assert sum(n for _, n in GROUPS) == H
SM_COST, DEP_LAT, K_AHEAD, SM_POS = 90.0, 90.0, 2, 0.5
PV_COST = (16.0, 8.5)
WV_PERIOD = 7
QV = tuple(range(2, NC, 3))
QV_BATCH = 2
FV = (5, 11)
WO_BLOCKS = 8
WD_BLOCKS = 2

bf16 = jnp.bfloat16
u32 = jnp.uint32
f32 = jnp.float32


def _nn(a, b):
    return jnp.dot(a, b, preferred_element_type=f32)


def _acc(a, t):
    return t if a is None else a + t


def _layernorm(xs):
    mean = jnp.sum(functools.reduce(jnp.add, xs), axis=1, keepdims=True) * (1.0 / D)
    cs = [x - mean for x in xs]
    var = jnp.sum(functools.reduce(jnp.add, [c * c for c in cs]), axis=1, keepdims=True) * (1.0 / D)
    inv = lax.rsqrt(var + EPS)
    return [c * inv for c in cs]


def _tile(c):
    return pl.ds(c * (LANES // 2), LANES // 2)


def _unpack(w):
    lo = pltpu.bitcast(w << 16, f32)
    hi = pltpu.bitcast(w & jnp.uint32(0xFFFF0000), f32)
    return lo, hi


def _emit(mxu, vpu):
    remaining, done = {}, {}
    for s in mxu + vpu:
        if s[2] is not None:
            remaining[s[2]] = remaining.get(s[2], 0) + 1
    t = [0.0, 0.0]
    idx = [0, 0]
    streams = (mxu, vpu)
    while idx[0] < len(mxu) or idx[1] < len(vpu):
        start = []
        for u in (0, 1):
            if idx[u] >= len(streams[u]):
                start.append(None)
                continue
            dep = streams[u][idx[u]][1]
            if dep is None or dep not in remaining:
                start.append(t[u])
            elif dep in done:
                start.append(max(t[u], done[dep] + DEP_LAT))
            else:
                start.append(None)
        u = min((u for u in (0, 1) if start[u] is not None), key=lambda u: start[u])
        cost, _, tag, fn = streams[u][idx[u]]
        idx[u] += 1
        fn()
        t[u] = start[u] + cost
        if tag is not None:
            remaining[tag] -= 1
            if remaining[tag] == 0:
                done[tag] = t[u]


def _kernel(x_h, wr_h, kT, vT, wq_h, wo_h, wg_h, wu_h, wd_h, o_ref,
            kbuf, vbuf, wq, wo, wg, wu, wd, x_v, wr_v, xs_ref, ys_ref, pbuf, xcol, qbd, hbuf,
            sems):

    k32, v32, wq32, wo32, wg32, wu32, wd32 = (
        r.bitcast(u32) for r in (kbuf, vbuf, wq, wo, wg, wu, wd))

    ksem = sems.at[0]
    wsem_q, wsem_x, wsem_o, wsem_f = sems.at[3], sems.at[4], sems.at[5], sems.at[6]

    def vsem_whole(b):
        return sems.at[1 + b % 2]

    def vsem_piece(p):
        return sems.at[2 + p]

    def ld(ref32, *idx):
        return pltpu.bitcast(ref32[idx], bf16)

    def col(j):
        return pl.ds(pl.multiple_of(S - W + LANES * j, LANES), LANES)

    def loop(n, fn):
        lax.fori_loop(0, n, lambda i, c: (fn(i), c)[1], 0)

    def start_k(b):
        loop(NJ, lambda j: pltpu.make_async_copy(kT.at[b, :, col(j)], kbuf.at[b, j], ksem).start())

    def wait_k(b):
        dst = kbuf.at[b]
        pltpu.make_async_copy(dst, dst, ksem).wait()

    def piece_rows(p):
        return pl.ds(PIECE_T0[p] * LANES, (PIECE_T0[p + 1] - PIECE_T0[p]) * LANES)

    def start_v_whole(b):
        loop(NJ, lambda j: pltpu.make_async_copy(vT.at[b, :, col(j)], vbuf.at[b, j], vsem_whole(b)).start())

    def wait_v_whole(b):
        dst = vbuf.at[b]
        pltpu.make_async_copy(dst, dst, vsem_whole(b)).wait()

    def start_v_piece(b, p):
        rows = piece_rows(p)
        loop(NJ, lambda j: pltpu.make_async_copy(
            vT.at[b, rows, col(j)], vbuf.at[b, j, rows], vsem_piece(p)).start())

    def wait_v_piece(b, p):
        dst = vbuf.at[b, :, piece_rows(p)]
        pltpu.make_async_copy(dst, dst, vsem_piece(p)).wait()

    def start_w(src, dst, n, sem):
        loop(n, lambda c: pltpu.make_async_copy(
            src.at[:, pl.ds(pl.multiple_of(LANES * c, LANES), LANES)], dst.at[c], sem).start())

    def start_tall(src, dst, nblk, sem):
        rows = src.shape[0] // nblk

        def fn(i):
            r = pl.ds(pl.multiple_of((i // ND) * rows, 16), rows)
            c = i % ND
            pltpu.make_async_copy(src.at[r, pl.ds(pl.multiple_of(LANES * c, LANES), LANES)],
                                  dst.at[c, r], sem).start()
        loop(nblk * ND, fn)

    def wait_w(dst, sem):
        pltpu.make_async_copy(dst, dst, sem).wait()

    x_cp = pltpu.make_async_copy(x_h, x_v, wsem_x)
    wr_cp = pltpu.make_async_copy(wr_h, wr_v, wsem_x)

    start_w(wq_h, wq, NC, wsem_q)
    x_cp.start()
    wr_cp.start()
    start_k(0)
    x_cp.wait()
    wr_cp.wait()

    xs_ref[...] = x_v[...].astype(f32)
    wr = wr_v[...].astype(f32).reshape(1, D)
    wr_t = [jnp.broadcast_to(wr[:, LANES * n:LANES * (n + 1)], (G, LANES)) for n in range(ND)]

    row = lax.broadcasted_iota(jnp.int32, (G, LANES), 0)
    lane = lax.broadcasted_iota(jnp.int32, (G, LANES), 1)

    def head_mask(c):
        colm = lane + c * LANES
        lo = row * DH
        return (colm >= lo) & (colm < lo + DH)

    wait_w(wq, wsem_q)
    start_v_whole(0)
    start_tall(wo_h, wo, WO_BLOCKS, wsem_o)
    start_w(wg_h, wg, NF, wsem_f)
    start_w(wu_h, wu, NF, wsem_f)
    start_tall(wd_h, wd, WD_BLOCKS, wsem_f)

    sub8 = lax.broadcasted_iota(jnp.int32, (8, LANES), 0)
    lane8 = lax.broadcasted_iota(jnp.int32, (8, LANES), 1)

    def to_columns(x_tiles):
        for n, t in enumerate(x_tiles):
            t = t[:8].astype(f32)
            for r in range(LANES // 8):
                xcol[n * (LANES // 8) + r] = jnp.broadcast_to(
                    jnp.sum(jnp.where(lane8 - sub8 == 8 * r, t, 0.0), axis=1, keepdims=True), (8, LANES))

    def vpu_matvec(cols):
        accs = [None] * len(cols)
        for kg in range(D // 16):
            x0, x1 = xcol[2 * kg], xcol[2 * kg + 1]
            for i, (w32, c) in enumerate(cols):
                w = ld(w32, c, pl.ds(kg * 8, 8), slice(None)).astype(f32)
                accs[i] = _acc(accs[i], w[:8] * x0 + w[8:] * x1)
        return [jnp.sum(a, axis=0, keepdims=True) for a in accs]

    def ffn(x1):
        xn = _layernorm(x1)
        xnb_t = [t.astype(bf16) for t in xn]
        xnb = jnp.concatenate(xnb_t, axis=1)
        rr = functools.reduce(jnp.add, [a.astype(f32) * w for a, w in zip(xnb_t, wr_t)])
        gate = jax.nn.sigmoid(jnp.sum(rr, axis=1, keepdims=True))
        to_columns(xnb_t)
        for f in range(NF):
            if f in FV:
                gt, ut = (jnp.broadcast_to(t, (G, LANES)) for t in vpu_matvec([(wg32, f), (wu32, f)]))
            else:
                gt = _nn(xnb, ld(wg32, f))
                ut = _nn(xnb, ld(wu32, f))
            hbuf[f] = (gt * jax.nn.sigmoid(gt) * ut).astype(bf16)
        y = [None] * ND
        for f in range(NF):
            h = hbuf[f]
            for n in range(ND):
                y[n] = _acc(y[n], _nn(h, ld(wd32, n, _tile(f), slice(None))))
        return [a + bb + c * gate for a, bb, c in zip(x1, xn, y)]

    diag = lane8 - 2 * sub8

    def tiles(gi):
        h0, nh = GROUPS[gi]
        return range(h0 * DH // LANES, (h0 + nh) * DH // LANES)

    def attention(b, xs, first):
        xlo, xhi = (b + B - 1) % B, (b + B - 2) % B
        xn = [t.astype(bf16) for t in _layernorm(xs)]
        xnb = jnp.concatenate(xn, axis=1)
        qv = {}

        to_columns(xn)
        for i in range(0, len(QV), QV_BATCH):
            part = QV[i:i + QV_BATCH]
            qv.update(zip(part, vpu_matvec([(wq32, cc) for cc in part])))
        for gi in range(len(GROUPS)):
            for c, cc in enumerate(tiles(gi)):
                qt = jnp.broadcast_to(qv[cc], (G, LANES)) if cc in qv else _nn(xnb, ld(wq32, cc))
                qbd[cc] = jnp.where(head_mask(c), qt, 0.0).astype(bf16)
        if first:
            l1_dma_start(b)

        st = {}
        mxu, vpu = [], []

        def qk_step(gi, cc, j, last):
            def fn():
                t = _nn(qbd[cc], ld(k32, b, j, _tile(cc), slice(None)))[:8]
                t = _acc(st.pop(('sc', gi, j), None), t)
                if last:
                    pbuf[gi, j] = t
                else:
                    st['sc', gi, j] = t
            return fn

        def sm_step(gi):
            def fn():
                sc = [pbuf[gi, j] for j in range(NJ)]
                m = jnp.max(functools.reduce(jnp.maximum, sc), axis=1, keepdims=True)
                es = [jnp.exp((t - m) * SCALE) for t in sc]
                l = jnp.sum(functools.reduce(jnp.add, es), axis=1, keepdims=True)
                inv = 1.0 / l
                for j in range(NJ):
                    pbuf[gi, j] = es[j] * inv
            return fn

        def pv_step(gi, r, rg):
            def fn():
                if rg == 0:
                    st['pb'] = [jnp.broadcast_to(pbuf[gi, j, r:r + 1, :], (8, LANES)) for j in range(NJ)]
                g16 = (GROUPS[gi][0] + r) * (DH // 16) + rg
                cc, k = divmod(g16, LANES // 16)
                rows = pl.ds(g16 * 8, 8)
                lo = hi = None
                for j in range(NJ):
                    if first:
                        a, c_ = _unpack(v32[b, j, rows, :])
                        k32[xlo, j, rows, :] = pltpu.bitcast(a, u32)
                        k32[xhi, j, rows, :] = pltpu.bitcast(c_, u32)
                    else:
                        a = pltpu.bitcast(k32[xlo, j, rows, :], f32)
                        c_ = pltpu.bitcast(k32[xhi, j, rows, :], f32)
                    lo = _acc(lo, a * st['pb'][j])
                    hi = _acc(hi, c_ * st['pb'][j])
                lo = jnp.sum(lo, axis=1, keepdims=True)
                hi = jnp.sum(hi, axis=1, keepdims=True)
                if vpu_wo(cc):
                    for n in range(ND):
                        a, c_ = _unpack(wo32[n, rows, :])
                        st['vacc', n] = _acc(st.get(('vacc', n)), a * lo + c_ * hi)
                else:
                    t = st.get(('ot', cc), jnp.zeros((8, LANES), f32))
                    t = jnp.where(diag == 16 * k, lo, t)
                    st['ot', cc] = jnp.where(diag == 16 * k + 1, hi, t)
            return fn

        def vpu_wo(cc):
            return (not first) and cc % WV_PERIOD == 0

        def wo_step(cc, n):
            def fn():
                if n == 0:
                    st['ot', cc] = st['ot', cc].astype(bf16)
                st['acc', n] = _acc(st.get(('acc', n)),
                                    _nn(st['ot', cc], ld(wo32, n, _tile(cc), slice(None))))
            return fn

        def wait_step(p):
            def fn():
                @pl.when(b == B - 1)
                def _():
                    wait_v_piece(b, p)

                if p == 0:
                    @pl.when(b < B - 1)
                    def _():
                        wait_v_whole(b)

                    @pl.when(b == 0)
                    def _():
                        wait_w(wo, wsem_o)
            return fn

        ng = len(GROUPS)
        pv_cost = PV_COST[0 if first else 1]
        if first:
            vpu += [(SM_COST, ('qk', gi), None, sm_step(gi)) for gi in range(ng)]
        else:
            vpu.append((SM_COST, ('qk', 0), None, sm_step(0)))
        for gi, (h0, nh) in enumerate(GROUPS):
            for r in range(nh):
                if not first and r == int(nh * SM_POS) and gi + 1 < ng:
                    vpu.append((SM_COST, ('qk', gi + 1), None, sm_step(gi + 1)))
                for rg in range(DH // 16):
                    g16 = (h0 + r) * (DH // 16) + rg
                    cc, k = divmod(g16, LANES // 16)
                    if first and k == 0 and cc in PIECE_T0[:-1]:
                        vpu.append((0.0, None, None, wait_step(PIECE_T0.index(cc))))
                    vpu.append((pv_cost + (8.0 if vpu_wo(cc) else 0.0), None, ('ot', cc), pv_step(gi, r, rg)))
        ahead = ng if first else K_AHEAD
        for gi in range(ng + ahead):
            if gi < ng:
                for cc in tiles(gi):
                    for j in range(NJ):
                        mxu.append((8, None, ('qk', gi), qk_step(gi, cc, j, cc == tiles(gi)[-1])))
            if gi >= ahead:
                for cc in tiles(gi - ahead):
                    for n in range(ND if not vpu_wo(cc) else 0):
                        mxu.append((8, ('ot', cc), None, wo_step(cc, n)))
        _emit(mxu, vpu)
        accs = [_acc(st.get(('vacc', n)), st['acc', n]) for n in range(ND)]
        return [x + jnp.sum(a, axis=0, keepdims=True) for x, a in zip(xs, accs)]

    def l1_dma_start(b):
        wait_k(b)

        @pl.when(b + 1 < B)
        def _():
            start_k(b + 1)

        @pl.when(b + 2 < B)
        def _():
            start_v_whole(b + 1)

        @pl.when(b + 2 == B)
        def _():
            for p in range(len(V_PIECES)):
                start_v_piece(b + 1, p)

    def layer(b, xs, first):
        x1 = attention(b, xs, first)
        if first:
            @pl.when(b == 0)
            def _():
                wait_w(wg, wsem_f)
                wait_w(wu, wsem_f)
                wait_w(wd, wsem_f)
        return ffn(x1)

    def batch(b, carry):
        x = jnp.broadcast_to(xs_ref[pl.ds(b, 1), :], (G, D))
        xs = [x[:, LANES * n:LANES * (n + 1)] for n in range(ND)]
        xs = layer(b, xs, True)
        xs = layer(b, xs, False)
        ys_ref[pl.ds(b, 1), :] = jnp.concatenate(xs, axis=1)[0:1, :]
        return carry

    lax.fori_loop(0, B, batch, 0)
    o_ref[...] = ys_ref[...].astype(o_ref.dtype)


@jax.jit
def pallas_interleave_layers__sliding_block_cached__moe_arch_mod__decode_kernel(
    A_x: jax.Array,
    A_k_cache: jax.Array,
    A_v_cache: jax.Array,
    A_wq: jax.Array,
    A_wo: jax.Array,
    B_x: jax.Array,
    B_w_r: jax.Array,
    B_w_gate: jax.Array,
    B_w_up: jax.Array,
    B_w_down: jax.Array,
):
    del B_x
    kT = jnp.swapaxes(A_k_cache, 2, 3).reshape(B, HD, S)
    vT = jnp.swapaxes(A_v_cache, 2, 3).reshape(B, HD, S)
    x = A_x.reshape(B, D)
    any_spec = pl.BlockSpec(memory_space=pl.ANY)
    out = pl.pallas_call(
        _kernel,
        in_specs=[any_spec] * 9,
        out_specs=pl.BlockSpec(memory_space=pltpu.VMEM),
        out_shape=jax.ShapeDtypeStruct((B, D), A_x.dtype),
        scratch_shapes=[
            pltpu.VMEM((B, NJ, HD, LANES), bf16),
            pltpu.VMEM((B, NJ, HD, LANES), bf16),
            pltpu.VMEM((NC, D, LANES), bf16),
            pltpu.VMEM((ND, HD, LANES), bf16),
            pltpu.VMEM((NF, D, LANES), bf16),
            pltpu.VMEM((NF, D, LANES), bf16),
            pltpu.VMEM((ND, F, LANES), bf16),
            pltpu.VMEM((B, D), bf16),
            pltpu.VMEM((D,), bf16),
            pltpu.VMEM((B, D), f32),
            pltpu.VMEM((B, D), f32),
            pltpu.VMEM((len(GROUPS), NJ, 8, LANES), f32),
            pltpu.VMEM((D // 8, 8, LANES), f32),
            pltpu.VMEM((NC, G, LANES), bf16),
            pltpu.VMEM((NF, G, LANES), bf16),
            pltpu.SemaphoreType.DMA((max(7, 2 + len(V_PIECES)),)),
        ],
        compiler_params=pltpu.CompilerParams(vmem_limit_bytes=126 * 1024 * 1024),
    )(x, B_w_r, kT, vT, A_wq, A_wo, B_w_gate, B_w_up, B_w_down)
    return out.reshape(A_x.shape)
```
